```python
import jax
import jax.numpy as jnp

def _softmax(x, axis=-1):
    return jax.nn.softmax(x, axis=axis)

def _gelu(x):
    return jax.nn.gelu(x, approximate=True)

def _silu(x):
    return jax.nn.silu(x)

def _sigmoid(x):
    return jax.nn.sigmoid(x)

def _layernorm(x, axis=-1, eps=1e-05):
    m = jnp.mean(x, axis=axis, keepdims=True)
    v = jnp.var(x, axis=axis, keepdims=True)
    return (x - m) / jnp.sqrt(v + eps)

def _scatter_add(tgt, idx, src, axis=0):
    return tgt.at[idx].add(src)

def _segment_sum(src, seg, n):
    return jax.ops.segment_sum(src, seg, n)

class _Rng:

    def __init__(self, key):
        self._k = key

    def _next(self):
        self._k, sub = jax.random.split(self._k)
        return sub

    def normal(self, shape):
        return jax.random.normal(self._next(), shape, dtype=jnp.bfloat16)

    def randint(self, lo, hi, shape):
        return jax.random.randint(self._next(), shape, lo, hi, dtype=jnp.int32)

    def uniform(self, shape, lo=0.0, hi=1.0):
        return jax.random.uniform(self._next(), shape, jnp.bfloat16, lo, hi)

    def permutation(self, n):
        return jax.random.permutation(self._next(), n)
kernel_name = 'recurrent_scan__memory_aug_recurrent_mem_tr__mixer_s_mlp__prompt'

def setup_inputs():
    _rng = _Rng(jax.random.key(int.from_bytes(__import__("os").urandom(4), "little")))
    _w = lambda a: (lambda t: t.astype(jnp.bfloat16) if jnp.issubdtype(t.dtype, jnp.floating) else t)(jnp.asarray(a))

    def _A_setup():
        B, S, Dm = (1, 2048, 1024)
        H, Dh = (32, 128)
        M, seg = (8, 32)
        seg = min(seg, S)
        S = S // seg * seg
        return {'x': _w((lambda *s: _rng.normal(s) * 0.05)(B, S, Dm)), 'mem0': _w((lambda *s: _rng.normal(s) * 0.05)(B, M, Dm)), 'Wq': _w((lambda *s: _rng.normal(s) * 0.05)(Dm, H, Dh) * Dm ** (-0.5)), 'Wk': _w((lambda *s: _rng.normal(s) * 0.05)(Dm, H, Dh) * Dm ** (-0.5)), 'Wv': _w((lambda *s: _rng.normal(s) * 0.05)(Dm, H, Dh) * Dm ** (-0.5)), 'Wo': _w((lambda *s: _rng.normal(s) * 0.05)(H, Dh, Dm) * (H * Dh) ** (-0.5)), 'seg_len': seg}
    _A_in = _A_setup()

    def _B_setup():
        B, S, D, F = (1, 2048, 1024, 3584)
        return {'x': _w((lambda *s: _rng.normal(s) * 0.05)(B, S, D)), 'w1': _w((lambda *s: _rng.normal(s) * 0.05)(D, D) * D ** (-0.5)), 'w2': _w((lambda *s: _rng.normal(s) * 0.05)(D, D) * D ** (-0.5)), 'w3': _w((lambda *s: _rng.normal(s) * 0.05)(D, F) * D ** (-0.5)), 'w4': _w((lambda *s: _rng.normal(s) * 0.05)(F, D) * F ** (-0.5))}
    _B_in = _B_setup()
    return {'A_x': _A_in['x'], 'A_mem0': _A_in['mem0'], 'A_Wq': _A_in['Wq'], 'A_Wk': _A_in['Wk'], 'A_Wv': _A_in['Wv'], 'A_Wo': _A_in['Wo'], 'A_seg_len': _A_in['seg_len'], 'B_x': _B_in['x'], 'B_w1': _B_in['w1'], 'B_w2': _B_in['w2'], 'B_w3': _B_in['w3'], 'B_w4': _B_in['w4']}

def reference(A_x, A_mem0, A_Wq, A_Wk, A_Wv, A_Wo, A_seg_len, B_x, B_w1, B_w2, B_w3, B_w4):

    def _A_ref(x, mem0, Wq, Wk, Wv, Wo, seg_len):
        B, S, Dm = x.shape
        H, Dh = (Wq.shape[1], Wq.shape[2])
        M = mem0.shape[1]
        scale = Dh ** (-0.5)
        n_seg = S // seg_len
        L = M + seg_len
        idx = jnp.arange(L)
        mask = (idx[:, None] < M) | (idx[:, None] >= idx[None, :])
        mem = mem0
        outs = []
        for s in range(n_seg):
            xs = x[:, s * seg_len:(s + 1) * seg_len, :].copy()
            h = jnp.concatenate([mem, xs], axis=1)
            q = jnp.einsum('btd,dhe->bhte', h, Wq)
            k = jnp.einsum('btd,dhe->bhte', h, Wk)
            v = jnp.einsum('btd,dhe->bhte', h, Wv)
            scores = jnp.einsum('bhqe,bhke->bhqk', q, k) * scale
            scores = jnp.where(mask[None, None], scores, -1000000000.0)
            p = _softmax(scores, axis=-1)
            o = jnp.einsum('bhqk,bhke->bhqe', p, v)
            o = jnp.einsum('bhte,hed->btd', o, Wo)
            mem = o[:, :M, :].copy()
            outs.append(o[:, M:, :])
        return jnp.concatenate(outs, axis=1)

    def _B_ref(x, w1, w2, w3, w4):
        B, S, D = x.shape
        h = _gelu(_layernorm(x, axis=-1) @ w1)
        c = D // 4
        g0 = jnp.pad(h[:, :, 0 * c:1 * c], ((0, 0), (1, 0), (0, 0)))[:, :S, :]
        g1 = jnp.pad(h[:, :, 1 * c:2 * c], ((0, 0), (0, 1), (0, 0)))[:, 1:, :]
        g2 = jnp.pad(h[:, :, 2 * c:3 * c], ((0, 0), (2, 0), (0, 0)))[:, :S, :]
        g3 = jnp.pad(h[:, :, 3 * c:], ((0, 0), (0, 2), (0, 0)))[:, 2:, :]
        hs = jnp.concatenate([g0, g1, g2, g3], axis=-1) @ w2
        x1 = x + hs
        h2 = _gelu(_layernorm(x1, axis=-1) @ w3) @ w4
        return x1 + h2
    x = A_x
    xn = _layernorm(x, axis=-1)
    s = _A_ref(xn, A_mem0, A_Wq, A_Wk, A_Wv, A_Wo, A_seg_len)
    g = _silu(_B_ref(xn, B_w1, B_w2, B_w3, B_w4))
    return x + s * g
```

```python
import functools

import jax
import jax.numpy as jnp
from jax import lax
import jax.experimental.pallas as pl
import jax.experimental.pallas.tpu as pltpu

_EPS = 1e-5
_HALO = 8
_F32 = jnp.float32
_BF16 = jnp.bfloat16
_U32 = jnp.uint32


def _layernorm(v):
    m = jnp.mean(v, axis=-1, keepdims=True)
    c = v - m
    var = jnp.mean(c * c, axis=-1, keepdims=True)
    return c * lax.rsqrt(var + _EPS)


def _gelu(v):
    inner = 0.7978845608028654 * (v + 0.044715 * (v * v * v))
    return 0.5 * v * (1.0 + jnp.tanh(inner))


def _silu(v):
    return v / (1.0 + jnp.exp(-v))


def _dot(a, b):
    return jnp.dot(a, b, preferred_element_type=_F32)


def _dot_nt(a, b):
    return lax.dot_general(a, b, (((1,), (1,)), ((), ())), preferred_element_type=_F32)


def _kernel(
    x_hbm, mem0_ref, wq_hbm, wk_hbm, wv_hbm, wo_hbm, w1_hbm, w2_hbm, w3_hbm, w4_hbm,
    out_hbm,
    x_v, o_v, xn_v, h_v, g_v, w1_v, w2_v, w3_v, w4_v, st_qkv, st_o, wqkv_v, wo_v,
    sem_x, sem_w, sem_st, sem_out,
    *, S, D, H, DH, M, SEG, TB,
):
    NB = S // TB
    DC = D // NB
    OC = H * DH // NB
    NP = H // 2
    L = M + SEG
    scale = DH ** (-0.5)

    def x_copy(i):
        rows = pl.ds(pl.multiple_of(i * TB, TB), TB)
        return pltpu.make_async_copy(x_hbm.at[rows], x_v.at[rows], sem_x.at[i])

    w_copies = [
        pltpu.make_async_copy(src, dst, sem_w.at[n])
        for n, (src, dst) in enumerate(
            ((w1_hbm, w1_v), (w2_hbm, w2_v), (w3_hbm, w3_v), (w4_hbm, w4_v)))
    ]

    def stage_copies(i, slot):
        rows = pl.ds(pl.multiple_of(i * (DC * H), DC * H), DC * H)
        cps = [
            pltpu.make_async_copy(w.at[rows], st_qkv.at[slot, n], sem_st.at[slot, n])
            for n, w in enumerate((wq_hbm, wk_hbm, wv_hbm))
        ]
        rows_o = pl.ds(pl.multiple_of(i * OC, OC), OC)
        cps.append(pltpu.make_async_copy(wo_hbm.at[rows_o], st_o.at[slot], sem_st.at[slot, 3]))
        return cps

    def out_copy(t):
        rows = pl.ds(pl.multiple_of(t * 2 * SEG, 2 * SEG), 2 * SEG)
        return pltpu.make_async_copy(o_v.at[rows], out_hbm.at[rows], sem_out.at[0])

    x_copy(0).start()
    w_copies[0].start()
    for i in range(1, NB):
        x_copy(i).start()

    zeros_halo = jnp.zeros((_HALO, D), _F32)
    h_v[pl.ds(0, _HALO), :] = zeros_halo
    h_v[pl.ds(_HALO + S, _HALO), :] = zeros_halo

    w_copies[0].wait()
    for cp in w_copies[1:]:
        cp.start()
    for cp in stage_copies(0, 0):
        cp.start()

    def phase1(i, carry):
        x_copy(i).wait()
        r0 = pl.multiple_of(i * TB, TB)
        xn = _layernorm(x_v[pl.ds(r0, TB), :].astype(_F32))
        xn_v[pl.ds(r0, TB), :] = xn
        hh = _gelu(_dot(_layernorm(xn).astype(_BF16), w1_v[...]))
        h_v[pl.ds(pl.multiple_of(r0 + _HALO, _HALO), TB), :] = hh
        return carry

    lax.fori_loop(0, NB, phase1, 0)

    for cp in w_copies[1:]:
        cp.wait()

    def repack(i, slot):
        st32 = st_qkv.bitcast(_U32)
        for n in range(3):
            src = st32.at[slot, n]
            for b in range(DC // 16):
                orow = pl.ds(pl.multiple_of(i * (DC // 2) + b * 8, 8), 8)
                for j in range(NP):
                    ev = src[pl.ds(b * 16 * NP + j, 8, stride=2 * NP), :]
                    od = src[pl.ds(b * 16 * NP + NP + j, 8, stride=2 * NP), :]
                    c0 = (6 * j + 2 * n) * DH
                    wqkv_v[orow, c0:c0 + DH] = (ev & _U32(0xFFFF)) | (od << 16)
                    wqkv_v[orow, c0 + DH:c0 + 2 * DH] = (ev >> 16) | (od & _U32(0xFFFF0000))
        rows = pl.ds(pl.multiple_of(i * (OC // 2), OC // 2), OC // 2)
        wo_v[rows, :] = pltpu.bitcast(st_o[slot], _U32)

    def phase2(i, carry):
        slot = i % 2

        @pl.when(i + 1 < NB)
        def _():
            for cp in stage_copies(i + 1, 1 - slot):
                cp.start()

        for cp in stage_copies(i, slot):
            cp.wait()

        r0 = pl.multiple_of(i * TB, TB)
        c = D // 4
        parts = []
        for q, shift in enumerate((-1, 1, -2, 2)):
            win = h_v[pl.ds(r0, TB + 2 * _HALO), q * c:(q + 1) * c]
            parts.append(win[_HALO + shift:_HALO + shift + TB].astype(_BF16))
        x1 = xn_v[pl.ds(r0, TB), :] + _dot(jnp.concatenate(parts, axis=1), w2_v[...])
        u = _gelu(_dot(_layernorm(x1).astype(_BF16), w3_v[...]))
        g_v[pl.ds(r0, TB), :] = _silu(x1 + _dot(u.astype(_BF16), w4_v[...]))
        repack(i, slot)
        return carry

    lax.fori_loop(0, NB, phase2, 0)

    row = lax.broadcasted_iota(jnp.int32, (2 * L, DH), 0)
    col = lax.broadcasted_iota(jnp.int32, (2 * L, DH), 1)
    rl = jnp.where(row >= L, row - L, row)
    cl = jnp.where(col >= L, col - L, col)
    same_head = ((row >= L) == (col >= L)) & (col < 2 * L)
    visible = same_head & ((rl < M) | (rl >= cl))
    fill = jnp.where(same_head, -1e9, -jnp.inf).astype(_F32)
    pad = jnp.zeros((DH - 2 * L, DH), _BF16)

    def project(lhs, j):
        w = pltpu.bitcast(wqkv_v[:, 6 * j * DH:6 * (j + 1) * DH], _BF16)
        return _dot(lhs, w)

    def pair(r, n):
        return jnp.concatenate(
            [r[:, 2 * n * DH:(2 * n + 1) * DH], r[:, (2 * n + 1) * DH:(2 * n + 2) * DH]],
            axis=0).astype(_BF16)

    def scores(r):
        s = _dot_nt(pair(r, 0), jnp.concatenate([pair(r, 1), pad], axis=0))
        return s, jnp.concatenate([pair(r, 2), pad], axis=0)

    def attend(s, v):
        z = jnp.where(visible, s * scale, fill)
        e = jnp.exp(z - jnp.max(z, axis=-1, keepdims=True))
        o = _dot(e.astype(_BF16), v) / jnp.sum(e, axis=-1, keepdims=True)
        return jnp.concatenate([o[:L], o[L:]], axis=1)

    def out_proj(o_parts, j0, j1):
        w = pltpu.bitcast(wo_v[j0 * DH:j1 * DH, :], _BF16)
        return _dot(jnp.concatenate(o_parts[j0:j1], axis=1), w)

    def step(lhs, seq_rows, out_rows):
        rs, sv, os_ = {}, {}, []
        for j in range(NP + 2):
            if j < NP:
                rs[j] = seq_rows(j, project(lhs, j))
            if 1 <= j <= NP:
                sv[j - 1] = scores(rs.pop(j - 1))
            if j >= 2:
                os_.append(out_rows(j - 2, attend(*sv.pop(j - 2))).astype(_BF16))
        split = NP * 3 // 4
        return out_proj(os_, 0, split) + out_proj(os_, split, NP)

    A = SEG + M
    B = SEG - M

    def phase3(t, mem):
        base = pl.multiple_of(t * 2 * SEG, 2 * SEG)
        held_r, held_o = {}, {}

        def seq_even(j, r):
            held_r[j] = r[L:]
            return r[:L]

        def out_even(j, o):
            held_o[j] = o[M + B:]
            return o[:M + B]

        def seq_odd(j, r):
            return jnp.concatenate([r[:M], held_r[j], r[M:]], axis=0)

        def out_odd(j, o):
            return jnp.concatenate([o[:M], held_o[j], o[M:]], axis=0)

        lhs0 = jnp.concatenate([mem, xn_v[pl.ds(base, A), :]], axis=0).astype(_BF16)
        y0 = step(lhs0, seq_even, out_even)
        rest = pl.ds(pl.multiple_of(base + A, 8), 2 * SEG - A)
        lhs1 = jnp.concatenate([y0[:M], xn_v[rest, :]], axis=0).astype(_BF16)
        y1 = step(lhs1, seq_odd, out_odd)

        rows = pl.ds(base, 2 * SEG)
        s = jnp.concatenate([y0[M:], y1[M:]], axis=0)
        o_v[rows, :] = (x_v[rows, :].astype(_F32) + s * g_v[rows, :]).astype(o_v.dtype)
        out_copy(t).start()
        return y1[:M]

    lax.fori_loop(0, S // (2 * SEG), phase3, mem0_ref[...].astype(_F32))
    pltpu.make_async_copy(o_v, out_hbm, sem_out.at[0]).wait()


@functools.partial(jax.jit, static_argnames=("A_seg_len",))
def pallas_recurrent_scan__memory_aug_recurrent_mem_tr__mixer_s_mlp__prompt_kernel(
    A_x: jax.Array,
    A_mem0: jax.Array,
    A_Wq: jax.Array,
    A_Wk: jax.Array,
    A_Wv: jax.Array,
    A_Wo: jax.Array,
    A_seg_len: int,
    B_x: jax.Array,
    B_w1: jax.Array,
    B_w2: jax.Array,
    B_w3: jax.Array,
    B_w4: jax.Array,
):
    del B_x
    batch, S, D = A_x.shape
    _, H, DH = A_Wq.shape
    M = A_mem0.shape[1]
    F = B_w3.shape[1]
    SEG = int(A_seg_len)
    TB = 256
    NB = S // TB
    assert batch == 1 and DH == 128 and M == 8 and SEG % 16 == 0 and 2 * (M + SEG) <= DH
    assert S % TB == 0 and S % (2 * SEG) == 0 and D % (16 * NB) == 0 and H % 2 == 0
    out_dtype = A_x.dtype

    hbm = pl.BlockSpec(memory_space=pl.ANY)
    out = pl.pallas_call(
        functools.partial(_kernel, S=S, D=D, H=H, DH=DH, M=M, SEG=SEG, TB=TB),
        out_shape=jax.ShapeDtypeStruct((S, D), out_dtype),
        in_specs=[hbm, pl.BlockSpec(memory_space=pltpu.VMEM)] + [hbm] * 8,
        out_specs=hbm,
        scratch_shapes=[
            pltpu.VMEM((S, D), _BF16),
            pltpu.VMEM((S, D), out_dtype),
            pltpu.VMEM((S, D), _F32),
            pltpu.VMEM((S + 2 * _HALO, D), _F32),
            pltpu.VMEM((S, D), _F32),
            pltpu.VMEM((D, D), _BF16),
            pltpu.VMEM((D, D), _BF16),
            pltpu.VMEM((D, F), _BF16),
            pltpu.VMEM((F, D), _BF16),
            pltpu.VMEM((2, 3, D // NB * H, DH), _BF16),
            pltpu.VMEM((2, H * DH // NB, D), _BF16),
            pltpu.VMEM((D // 2, 3 * H * DH), _U32),
            pltpu.VMEM((H * DH // 2, D), _U32),
            pltpu.SemaphoreType.DMA((NB,)),
            pltpu.SemaphoreType.DMA((4,)),
            pltpu.SemaphoreType.DMA((2, 4)),
            pltpu.SemaphoreType.DMA((1,)),
        ],
        compiler_params=pltpu.CompilerParams(vmem_limit_bytes=120 * 1024 * 1024),
    )(
        A_x.reshape(S, D),
        A_mem0.reshape(M, D),
        A_Wq.reshape(D * H, DH),
        A_Wk.reshape(D * H, DH),
        A_Wv.reshape(D * H, DH),
        A_Wo.reshape(H * DH, D),
        B_w1, B_w2, B_w3, B_w4,
    )
    return out.reshape(batch, S, D)
```

```python
import functools

import jax
import jax.numpy as jnp
from jax import lax
import jax.experimental.pallas as pl
import jax.experimental.pallas.tpu as pltpu

_EPS = 1e-5
_HALO = 8
_F32 = jnp.float32
_BF16 = jnp.bfloat16
_U32 = jnp.uint32


def _layernorm(v):
    m = jnp.mean(v, axis=-1, keepdims=True)
    c = v - m
    var = jnp.mean(c * c, axis=-1, keepdims=True)
    return c * lax.rsqrt(var + _EPS)


def _gelu(v):
    inner = 0.7978845608028654 * (v + 0.044715 * (v * v * v))
    return 0.5 * v * (1.0 + jnp.tanh(inner))


def _silu(v):
    return v / (1.0 + jnp.exp(-v))


def _dot(a, b):
    return jnp.dot(a, b, preferred_element_type=_F32)


def _dot_nt(a, b):
    return lax.dot_general(a, b, (((1,), (1,)), ((), ())), preferred_element_type=_F32)


def _kernel(
    x_hbm, mem0_ref, wq_hbm, wk_hbm, wv_hbm, wo_hbm, w1_hbm, w2_hbm, w3_hbm, w4_hbm,
    out_hbm,
    x_v, o_v, xn_v, h_v, g_v, w1_v, w2_v, w3_v, w4_v, st_qkv, st_o, wqkv_v, wo_v,
    sem_x, sem_w, sem_st, sem_out,
    *, S, D, H, DH, M, SEG, TB,
):
    NB = S // TB
    DC = D // NB
    OC = H * DH // NB
    NP = H // 2
    L = M + SEG
    scale = DH ** (-0.5)

    def x_copy(i):
        rows = pl.ds(pl.multiple_of(i * TB, TB), TB)
        return pltpu.make_async_copy(x_hbm.at[rows], x_v.at[rows], sem_x.at[i])

    w_copies = [
        pltpu.make_async_copy(src, dst, sem_w.at[n])
        for n, (src, dst) in enumerate(
            ((w1_hbm, w1_v), (w2_hbm, w2_v), (w3_hbm, w3_v), (w4_hbm, w4_v)))
    ]

    def stage_copies(i, slot):
        rows = pl.ds(pl.multiple_of(i * (DC * H), DC * H), DC * H)
        cps = [
            pltpu.make_async_copy(w.at[rows], st_qkv.at[slot, n], sem_st.at[slot, n])
            for n, w in enumerate((wq_hbm, wk_hbm, wv_hbm))
        ]
        rows_o = pl.ds(pl.multiple_of(i * OC, OC), OC)
        cps.append(pltpu.make_async_copy(wo_hbm.at[rows_o], st_o.at[slot], sem_st.at[slot, 3]))
        return cps

    def out_copy(t):
        rows = pl.ds(pl.multiple_of(t * 2 * SEG, 2 * SEG), 2 * SEG)
        return pltpu.make_async_copy(o_v.at[rows], out_hbm.at[rows], sem_out.at[0])

    x_copy(0).start()
    w_copies[0].start()
    for i in range(1, NB):
        x_copy(i).start()

    zeros_halo = jnp.zeros((_HALO, D), _F32)
    h_v[pl.ds(0, _HALO), :] = zeros_halo
    h_v[pl.ds(_HALO + S, _HALO), :] = zeros_halo

    w_copies[0].wait()
    for cp in w_copies[1:]:
        cp.start()
    for cp in stage_copies(0, 0):
        cp.start()

    def phase1(i, carry):
        x_copy(i).wait()
        r0 = pl.multiple_of(i * TB, TB)
        xn = _layernorm(x_v[pl.ds(r0, TB), :].astype(_F32))
        xn_v[pl.ds(r0, TB), :] = xn
        hh = _gelu(_dot(_layernorm(xn).astype(_BF16), w1_v[...]))
        h_v[pl.ds(pl.multiple_of(r0 + _HALO, _HALO), TB), :] = hh
        return carry

    lax.fori_loop(0, NB, phase1, 0)

    for cp in w_copies[1:]:
        cp.wait()

    def repack(i, slot):
        st32 = st_qkv.bitcast(_U32)
        for n in range(3):
            src = st32.at[slot, n]
            for b in range(DC // 16):
                orow = pl.ds(pl.multiple_of(i * (DC // 2) + b * 8, 8), 8)
                for j in range(NP):
                    ev = src[pl.ds(b * 16 * NP + j, 8, stride=2 * NP), :]
                    od = src[pl.ds(b * 16 * NP + NP + j, 8, stride=2 * NP), :]
                    c0 = (6 * j + 2 * n) * DH
                    wqkv_v[orow, c0:c0 + DH] = (ev & _U32(0xFFFF)) | (od << 16)
                    wqkv_v[orow, c0 + DH:c0 + 2 * DH] = (ev >> 16) | (od & _U32(0xFFFF0000))
        rows = pl.ds(pl.multiple_of(i * (OC // 2), OC // 2), OC // 2)
        wo_v[rows, :] = pltpu.bitcast(st_o[slot], _U32)

    def phase2(i, carry):
        slot = i % 2

        @pl.when(i + 1 < NB)
        def _():
            for cp in stage_copies(i + 1, 1 - slot):
                cp.start()

        for cp in stage_copies(i, slot):
            cp.wait()

        r0 = pl.multiple_of(i * TB, TB)
        c = D // 4
        parts = []
        for q, shift in enumerate((-1, 1, -2, 2)):
            win = h_v[pl.ds(r0, TB + 2 * _HALO), q * c:(q + 1) * c]
            parts.append(win[_HALO + shift:_HALO + shift + TB].astype(_BF16))
        x1 = xn_v[pl.ds(r0, TB), :] + _dot(jnp.concatenate(parts, axis=1), w2_v[...])
        u = _gelu(_dot(_layernorm(x1).astype(_BF16), w3_v[...]))
        g_v[pl.ds(r0, TB), :] = _silu(x1 + _dot(u.astype(_BF16), w4_v[...]))
        repack(i, slot)
        return carry

    lax.fori_loop(0, NB, phase2, 0)

    row = lax.broadcasted_iota(jnp.int32, (2 * L, DH), 0)
    col = lax.broadcasted_iota(jnp.int32, (2 * L, DH), 1)
    rl = jnp.where(row >= L, row - L, row)
    cl = jnp.where(col >= L, col - L, col)
    same_head = ((row >= L) == (col >= L)) & (col < 2 * L)
    visible = same_head & ((rl < M) | (rl >= cl))
    fill = jnp.where(same_head, -1e9, -jnp.inf).astype(_F32)
    pad = jnp.zeros((DH - 2 * L, DH), _BF16)

    def project(lhs, j):
        w = pltpu.bitcast(wqkv_v[:, 6 * j * DH:6 * (j + 1) * DH], _BF16)
        return _dot(lhs, w)

    def pair(r, n):
        return jnp.concatenate(
            [r[:, 2 * n * DH:(2 * n + 1) * DH], r[:, (2 * n + 1) * DH:(2 * n + 2) * DH]],
            axis=0).astype(_BF16)

    def scores(r):
        s = _dot_nt(pair(r, 0), jnp.concatenate([pair(r, 1), pad], axis=0))
        return s, jnp.concatenate([pair(r, 2), pad], axis=0)

    def attend(s, v):
        z = jnp.where(visible, s * scale, fill)
        e = jnp.exp(z - jnp.max(z, axis=-1, keepdims=True))
        p = e / jnp.sum(e, axis=-1, keepdims=True)
        o = _dot(p.astype(_BF16), v)
        return jnp.concatenate([o[:L], o[L:]], axis=1)

    def out_proj(o, j0, j1, n0, n1):
        return _dot(o, pltpu.bitcast(wo_v[j0 * DH:j1 * DH, n0:n1], _BF16))

    def step(lhs, seq_rows, out_rows):
        LAG = 3
        early = NP - LAG
        nw = D // (LAG + 1)
        rs, sv, os_, ys = {}, {}, [], []
        for j in range(NP + LAG + 1):
            if j < NP:
                rs[j] = seq_rows(j, project(lhs, j))
            else:
                if j == NP:
                    o_early = jnp.concatenate(os_[:early], axis=1)
                ys.append(out_proj(o_early, 0, early, (j - NP) * nw, (j - NP + 1) * nw))
            if 1 <= j <= NP:
                sv[j - 1] = scores(rs.pop(j - 1))
            if LAG <= j < NP + LAG:
                os_.append(out_rows(j - LAG, attend(*sv.pop(j - LAG))).astype(_BF16))
        o_late = jnp.concatenate(os_[early:], axis=1)
        return jnp.concatenate(ys, axis=1) + out_proj(o_late, early, NP, 0, D)

    A = SEG + M
    B = SEG - M

    def phase3(t, mem):
        base = pl.multiple_of(t * 2 * SEG, 2 * SEG)
        held_r, held_o = {}, {}

        def seq_even(j, r):
            held_r[j] = r[L:]
            return r[:L]

        def out_even(j, o):
            held_o[j] = o[M + B:]
            return o[:M + B]

        def seq_odd(j, r):
            return jnp.concatenate([r[:M], held_r[j], r[M:]], axis=0)

        def out_odd(j, o):
            return jnp.concatenate([o[:M], held_o[j], o[M:]], axis=0)

        lhs0 = jnp.concatenate([mem, xn_v[pl.ds(base, A), :]], axis=0).astype(_BF16)
        y0 = step(lhs0, seq_even, out_even)
        rest = pl.ds(pl.multiple_of(base + A, 8), 2 * SEG - A)
        lhs1 = jnp.concatenate([y0[:M], xn_v[rest, :]], axis=0).astype(_BF16)
        y1 = step(lhs1, seq_odd, out_odd)

        rows = pl.ds(base, 2 * SEG)
        s = jnp.concatenate([y0[M:], y1[M:]], axis=0)
        o_v[rows, :] = (x_v[rows, :].astype(_F32) + s * g_v[rows, :]).astype(o_v.dtype)
        out_copy(t).start()
        return y1[:M]

    lax.fori_loop(0, S // (2 * SEG), phase3, mem0_ref[...].astype(_F32))
    pltpu.make_async_copy(o_v, out_hbm, sem_out.at[0]).wait()


@functools.partial(jax.jit, static_argnames=("A_seg_len",))
def pallas_recurrent_scan__memory_aug_recurrent_mem_tr__mixer_s_mlp__prompt_kernel(
    A_x: jax.Array,
    A_mem0: jax.Array,
    A_Wq: jax.Array,
    A_Wk: jax.Array,
    A_Wv: jax.Array,
    A_Wo: jax.Array,
    A_seg_len: int,
    B_x: jax.Array,
    B_w1: jax.Array,
    B_w2: jax.Array,
    B_w3: jax.Array,
    B_w4: jax.Array,
):
    del B_x
    batch, S, D = A_x.shape
    _, H, DH = A_Wq.shape
    M = A_mem0.shape[1]
    F = B_w3.shape[1]
    SEG = int(A_seg_len)
    TB = 256
    NB = S // TB
    assert batch == 1 and DH == 128 and M == 8 and SEG % 16 == 0 and 2 * (M + SEG) <= DH
    assert S % TB == 0 and S % (2 * SEG) == 0 and D % (16 * NB) == 0 and H % 2 == 0
    out_dtype = A_x.dtype

    hbm = pl.BlockSpec(memory_space=pl.ANY)
    out = pl.pallas_call(
        functools.partial(_kernel, S=S, D=D, H=H, DH=DH, M=M, SEG=SEG, TB=TB),
        out_shape=jax.ShapeDtypeStruct((S, D), out_dtype),
        in_specs=[hbm, pl.BlockSpec(memory_space=pltpu.VMEM)] + [hbm] * 8,
        out_specs=hbm,
        scratch_shapes=[
            pltpu.VMEM((S, D), _BF16),
            pltpu.VMEM((S, D), out_dtype),
            pltpu.VMEM((S, D), _F32),
            pltpu.VMEM((S + 2 * _HALO, D), _F32),
            pltpu.VMEM((S, D), _F32),
            pltpu.VMEM((D, D), _BF16),
            pltpu.VMEM((D, D), _BF16),
            pltpu.VMEM((D, F), _BF16),
            pltpu.VMEM((F, D), _BF16),
            pltpu.VMEM((2, 3, D // NB * H, DH), _BF16),
            pltpu.VMEM((2, H * DH // NB, D), _BF16),
            pltpu.VMEM((D // 2, 3 * H * DH), _U32),
            pltpu.VMEM((H * DH // 2, D), _U32),
            pltpu.SemaphoreType.DMA((NB,)),
            pltpu.SemaphoreType.DMA((4,)),
            pltpu.SemaphoreType.DMA((2, 4)),
            pltpu.SemaphoreType.DMA((1,)),
        ],
        compiler_params=pltpu.CompilerParams(vmem_limit_bytes=120 * 1024 * 1024),
    )(
        A_x.reshape(S, D),
        A_mem0.reshape(M, D),
        A_Wq.reshape(D * H, DH),
        A_Wk.reshape(D * H, DH),
        A_Wv.reshape(D * H, DH),
        A_Wo.reshape(H * DH, D),
        B_w1, B_w2, B_w3, B_w4,
    )
    return out.reshape(batch, S, D)
```

```python
import functools

import jax
import jax.numpy as jnp
from jax import lax
import jax.experimental.pallas as pl
import jax.experimental.pallas.tpu as pltpu

_EPS = 1e-5
_HALO = 8
_F32 = jnp.float32
_BF16 = jnp.bfloat16
_U32 = jnp.uint32


def _layernorm(v):
    m = jnp.mean(v, axis=-1, keepdims=True)
    c = v - m
    var = jnp.mean(c * c, axis=-1, keepdims=True)
    return c * lax.rsqrt(var + _EPS)


def _gelu(v):
    inner = 0.7978845608028654 * (v + 0.044715 * (v * v * v))
    return 0.5 * v * (1.0 + jnp.tanh(inner))


def _silu(v):
    return v / (1.0 + jnp.exp(-v))


def _dot(a, b):
    return jnp.dot(a, b, preferred_element_type=_F32)


def _dot_nt(a, b):
    return lax.dot_general(a, b, (((1,), (1,)), ((), ())), preferred_element_type=_F32)


def _kernel(
    x_hbm, mem0_ref, wq_hbm, wk_hbm, wv_hbm, wo_hbm, w1_hbm, w2_hbm, w3_hbm, w4_hbm,
    out_hbm,
    x_v, o_v, xn_v, h_v, g_v, lhs_v, w1_v, w2_v, w3_v, w4_v, wqkv_v, wo_v,
    sem_x, sem_w, sem_qkv, sem_out,
    *, S, D, H, DH, M, SEG, TB,
):
    NB = S // TB
    NP = H // 2
    PG = NP // NB
    L = M + SEG
    scale = DH ** (-0.5)

    def weights(ref):
        return pltpu.bitcast(ref, _BF16)

    def chunk(i, offset=0):
        return pl.ds(pl.multiple_of(i * TB + offset, 8), TB)

    def x_copy(i):
        rows = pl.ds(pl.multiple_of(i * TB, TB), TB)
        return pltpu.make_async_copy(x_hbm.at[rows], x_v.at[rows], sem_x.at[i])

    w_copies = [
        pltpu.make_async_copy(src, dst.bitcast(_BF16), sem_w.at[n])
        for n, (src, dst) in enumerate(
            ((w1_hbm, w1_v), (w2_hbm, w2_v), (w3_hbm, w3_v), (w4_hbm, w4_v), (wo_hbm, wo_v)))
    ]

    def start_group(i):
        for n, w in enumerate((wq_hbm, wk_hbm, wv_hbm)):
            w32 = w.bitcast(_U32)
            for p in range(PG):
                for parity in range(2):
                    c0 = (6 * p + 2 * n + parity) * DH
                    pltpu.make_async_copy(
                        w32.at[:, parity, i * PG + p, :],
                        wqkv_v.at[i, :, pl.ds(c0, DH)],
                        sem_qkv.at[i]).start()

    def repack(i):
        for c0 in range(0, 6 * PG * DH, 2 * DH):
            ev = wqkv_v[i, :, c0:c0 + DH]
            od = wqkv_v[i, :, c0 + DH:c0 + 2 * DH]
            wqkv_v[i, :, c0:c0 + DH] = (ev & _U32(0xFFFF)) | (od << 16)
            wqkv_v[i, :, c0 + DH:c0 + 2 * DH] = (ev >> 16) | (od & _U32(0xFFFF0000))

    def out_copy(t):
        rows = pl.ds(pl.multiple_of(t * 2 * SEG, 2 * SEG), 2 * SEG)
        return pltpu.make_async_copy(o_v.at[rows], out_hbm.at[rows], sem_out.at[0])

    x_copy(0).start()
    w_copies[0].start()
    for i in range(1, NB):
        x_copy(i).start()
    for cp in w_copies[1:4]:
        cp.start()

    zeros_halo = jnp.zeros((_HALO, D), _F32)
    h_v[pl.ds(0, _HALO), :] = zeros_halo
    h_v[pl.ds(_HALO + S, _HALO), :] = zeros_halo

    def norm_x(i, slot):
        xn = _layernorm(x_v[chunk(i), :].astype(_F32))
        xn_v[chunk(i), :] = xn
        lhs_v[slot] = _layernorm(xn).astype(_BF16)

    x_copy(0).wait()
    norm_x(0, 0)
    w_copies[0].wait()

    def phase1(i, carry):
        @pl.when(i + 1 < NB)
        def _():
            x_copy(i + 1).wait()

        h_v[chunk(i, _HALO), :] = _gelu(_dot(lhs_v[i % 2], weights(w1_v[...])))
        norm_x(jnp.minimum(i + 1, NB - 1), (i + 1) % 2)
        return carry

    lax.fori_loop(0, NB, phase1, 0)

    w_copies[1].wait()

    def phase2a(i, carry):
        start_group(i)
        c = D // 4
        parts = []
        for q, shift in enumerate((-1, 1, -2, 2)):
            win = h_v[pl.ds(pl.multiple_of(i * TB, TB), TB + 2 * _HALO), q * c:(q + 1) * c]
            parts.append(win[_HALO + shift:_HALO + shift + TB].astype(_BF16))
        hs = _dot(jnp.concatenate(parts, axis=1), weights(w2_v[...]))
        g_v[chunk(i), :] = xn_v[chunk(i), :] + hs
        return carry

    lax.fori_loop(0, NB, phase2a, 0)
    w_copies[4].start()

    def norm_x1(i, slot):
        lhs_v[slot] = _layernorm(g_v[chunk(i), :]).astype(_BF16)

    norm_x1(0, 0)
    w_copies[2].wait()
    w_copies[3].wait()

    def phase2b(i, carry):
        pltpu.make_async_copy(wqkv_v.at[i], wqkv_v.at[i], sem_qkv.at[i]).wait()
        u = _gelu(_dot(lhs_v[i % 2], weights(w3_v[...])))
        norm_x1(jnp.minimum(i + 1, NB - 1), (i + 1) % 2)
        g_v[chunk(i), :] = _silu(g_v[chunk(i), :] + _dot(u.astype(_BF16), weights(w4_v[...])))
        repack(i)
        return carry

    lax.fori_loop(0, NB, phase2b, 0)
    w_copies[4].wait()

    row = lax.broadcasted_iota(jnp.int32, (2 * L, DH), 0)
    col = lax.broadcasted_iota(jnp.int32, (2 * L, DH), 1)
    rl = jnp.where(row >= L, row - L, row)
    cl = jnp.where(col >= L, col - L, col)
    same_head = ((row >= L) == (col >= L)) & (col < 2 * L)
    visible = same_head & ((rl < M) | (rl >= cl))
    fill = jnp.where(same_head, -1e9, -jnp.inf).astype(_F32)
    pad = jnp.zeros((DH - 2 * L, DH), _BF16)

    def project(lhs, j):
        c0 = 6 * (j % PG) * DH
        return _dot(lhs, weights(wqkv_v[j // PG, :, c0:c0 + 6 * DH]))

    def pair(r, n):
        return jnp.concatenate(
            [r[:, 2 * n * DH:(2 * n + 1) * DH], r[:, (2 * n + 1) * DH:(2 * n + 2) * DH]],
            axis=0).astype(_BF16)

    def scores(r):
        s = _dot_nt(pair(r, 0), jnp.concatenate([pair(r, 1), pad], axis=0))
        return s, jnp.concatenate([pair(r, 2), pad], axis=0)

    def attend(s, v):
        z = jnp.where(visible, s * scale, fill)
        e = jnp.exp(z - jnp.max(z, axis=-1, keepdims=True))
        p = e / jnp.sum(e, axis=-1, keepdims=True)
        o = _dot(p.astype(_BF16), v)
        return jnp.concatenate([o[:L], o[L:]], axis=1)

    def out_proj(o, j0, j1, n0, n1):
        return _dot(o, weights(wo_v[j0 * DH:j1 * DH, n0:n1]))

    def step(lhs, seq_rows, out_rows):
        LAG = 3
        early = NP - LAG
        nw = D // (LAG + 1)
        rs, sv, os_, ys = {}, {}, [], []
        for j in range(NP + LAG + 1):
            if j < NP:
                rs[j] = seq_rows(j, project(lhs, j))
            else:
                if j == NP:
                    o_early = jnp.concatenate(os_[:early], axis=1)
                ys.append(out_proj(o_early, 0, early, (j - NP) * nw, (j - NP + 1) * nw))
            if 1 <= j <= NP:
                sv[j - 1] = scores(rs.pop(j - 1))
            if LAG <= j < NP + LAG:
                os_.append(out_rows(j - LAG, attend(*sv.pop(j - LAG))).astype(_BF16))
        o_late = jnp.concatenate(os_[early:], axis=1)
        return jnp.concatenate(ys, axis=1) + out_proj(o_late, early, NP, 0, D)

    A = SEG + M
    B = SEG - M

    def phase3(t, mem):
        base = pl.multiple_of(t * 2 * SEG, 2 * SEG)
        held_r, held_o = {}, {}

        def seq_even(j, r):
            held_r[j] = r[L:]
            return r[:L]

        def out_even(j, o):
            held_o[j] = o[M + B:]
            return o[:M + B]

        def seq_odd(j, r):
            return jnp.concatenate([r[:M], held_r[j], r[M:]], axis=0)

        def out_odd(j, o):
            return jnp.concatenate([o[:M], held_o[j], o[M:]], axis=0)

        lhs0 = jnp.concatenate([mem, xn_v[pl.ds(base, A), :]], axis=0).astype(_BF16)
        y0 = step(lhs0, seq_even, out_even)
        rest = pl.ds(pl.multiple_of(base + A, 8), 2 * SEG - A)
        lhs1 = jnp.concatenate([y0[:M], xn_v[rest, :]], axis=0).astype(_BF16)
        y1 = step(lhs1, seq_odd, out_odd)

        rows = pl.ds(base, 2 * SEG)
        s = jnp.concatenate([y0[M:], y1[M:]], axis=0)
        o_v[rows, :] = (x_v[rows, :].astype(_F32) + s * g_v[rows, :]).astype(o_v.dtype)
        out_copy(t).start()
        return y1[:M]

    lax.fori_loop(0, S // (2 * SEG), phase3, mem0_ref[...].astype(_F32))
    pltpu.make_async_copy(o_v, out_hbm, sem_out.at[0]).wait()


@functools.partial(jax.jit, static_argnames=("A_seg_len",))
def pallas_recurrent_scan__memory_aug_recurrent_mem_tr__mixer_s_mlp__prompt_kernel(
    A_x: jax.Array,
    A_mem0: jax.Array,
    A_Wq: jax.Array,
    A_Wk: jax.Array,
    A_Wv: jax.Array,
    A_Wo: jax.Array,
    A_seg_len: int,
    B_x: jax.Array,
    B_w1: jax.Array,
    B_w2: jax.Array,
    B_w3: jax.Array,
    B_w4: jax.Array,
):
    del B_x
    batch, S, D = A_x.shape
    _, H, DH = A_Wq.shape
    M = A_mem0.shape[1]
    F = B_w3.shape[1]
    SEG = int(A_seg_len)
    TB = 256
    NB = S // TB
    assert batch == 1 and DH == 128 and M == 8 and SEG % 16 == 0 and 2 * (M + SEG) <= DH
    assert S % TB == 0 and S % (2 * SEG) == 0 and D % (16 * NB) == 0 and H % 2 == 0
    out_dtype = A_x.dtype

    hbm = pl.BlockSpec(memory_space=pl.ANY)
    out = pl.pallas_call(
        functools.partial(_kernel, S=S, D=D, H=H, DH=DH, M=M, SEG=SEG, TB=TB),
        out_shape=jax.ShapeDtypeStruct((S, D), out_dtype),
        in_specs=[hbm, pl.BlockSpec(memory_space=pltpu.VMEM)] + [hbm] * 8,
        out_specs=hbm,
        scratch_shapes=[
            pltpu.VMEM((S, D), _BF16),
            pltpu.VMEM((S, D), out_dtype),
            pltpu.VMEM((S, D), _F32),
            pltpu.VMEM((S + 2 * _HALO, D), _F32),
            pltpu.VMEM((S, D), _F32),
            pltpu.VMEM((2, TB, D), _BF16),
            pltpu.VMEM((D // 2, D), _U32),
            pltpu.VMEM((D // 2, D), _U32),
            pltpu.VMEM((D // 2, F), _U32),
            pltpu.VMEM((F // 2, D), _U32),
            pltpu.VMEM((NB, D // 2, 3 * H * DH // NB), _U32),
            pltpu.VMEM((H * DH // 2, D), _U32),
            pltpu.SemaphoreType.DMA((NB,)),
            pltpu.SemaphoreType.DMA((5,)),
            pltpu.SemaphoreType.DMA((NB,)),
            pltpu.SemaphoreType.DMA((1,)),
        ],
        compiler_params=pltpu.CompilerParams(vmem_limit_bytes=120 * 1024 * 1024),
    )(
        A_x.reshape(S, D),
        A_mem0.reshape(M, D),
        A_Wq.reshape(D // 2, 2, H, DH),
        A_Wk.reshape(D // 2, 2, H, DH),
        A_Wv.reshape(D // 2, 2, H, DH),
        A_Wo.reshape(H * DH, D),
        B_w1, B_w2, B_w3, B_w4,
    )
    return out.reshape(batch, S, D)
```

```python
import functools

import jax
import jax.numpy as jnp
from jax import lax
import jax.experimental.pallas as pl
import jax.experimental.pallas.tpu as pltpu

_EPS = 1e-5
_HALO = 8
_F32 = jnp.float32
_BF16 = jnp.bfloat16
_U32 = jnp.uint32


def _layernorm(v):
    m = jnp.mean(v, axis=-1, keepdims=True)
    c = v - m
    var = jnp.mean(c * c, axis=-1, keepdims=True)
    return c * lax.rsqrt(var + _EPS)


def _gelu(v):
    inner = 0.7978845608028654 * (v + 0.044715 * (v * v * v))
    return 0.5 * v * (1.0 + jnp.tanh(inner))


def _silu(v):
    return v / (1.0 + jnp.exp(-v))


def _dot(a, b):
    return jnp.dot(a, b, preferred_element_type=_F32)


def _dot_nt(a, b):
    return lax.dot_general(a, b, (((1,), (1,)), ((), ())), preferred_element_type=_F32)


def _kernel(
    x_hbm, mem0_ref, wq_hbm, wk_hbm, wv_hbm, wo_hbm, w1_hbm, w2_hbm, w3_hbm, w4_hbm,
    out_hbm,
    x_v, o_v, xn_v, h_v, g_v, lhs_v, w1_v, w2_v, w3_v, w4_v, wqkv_v, wo_v,
    sem_x, sem_w, sem_qkv, sem_out,
    *, S, D, H, DH, F, M, SEG, TB,
):
    NB = S // TB
    NP = H // 2
    PG = NP // NB
    L = M + SEG
    scale = DH ** (-0.5)

    def weights(ref):
        return pltpu.bitcast(ref, _BF16)

    def chunk(i, offset=0):
        return pl.ds(pl.multiple_of(i * TB + offset, 8), TB)

    def x_copy(i):
        rows = pl.ds(pl.multiple_of(i * TB, TB), TB)
        return pltpu.make_async_copy(x_hbm.at[rows], x_v.at[rows], sem_x.at[i])

    w_copies = [
        pltpu.make_async_copy(src, dst.bitcast(_BF16), sem_w.at[n])
        for n, (src, dst) in enumerate(
            ((w1_hbm, w1_v), (w2_hbm, w2_v), (w3_hbm, w3_v), (w4_hbm, w4_v), (wo_hbm, wo_v)))
    ]

    def start_group(i):
        for n, w in enumerate((wq_hbm, wk_hbm, wv_hbm)):
            w32 = w.bitcast(_U32)
            for p in range(PG):
                for parity in range(2):
                    c0 = (6 * p + 2 * n + parity) * DH
                    pltpu.make_async_copy(
                        w32.at[:, parity, i * PG + p, :],
                        wqkv_v.at[i, :, pl.ds(c0, DH)],
                        sem_qkv.at[i]).start()

    def repack(i):
        for c0 in range(0, 6 * PG * DH, 2 * DH):
            for r0 in range(0, D // 2, 8):
                rows = slice(r0, r0 + 8)
                ev = wqkv_v[i, rows, c0:c0 + DH]
                od = wqkv_v[i, rows, c0 + DH:c0 + 2 * DH]
                wqkv_v[i, rows, c0:c0 + DH] = (ev & _U32(0xFFFF)) | (od << 16)
                wqkv_v[i, rows, c0 + DH:c0 + 2 * DH] = (ev >> 16) | (od & _U32(0xFFFF0000))

    def out_copy(t):
        rows = pl.ds(pl.multiple_of(t * 2 * SEG, 2 * SEG), 2 * SEG)
        return pltpu.make_async_copy(o_v.at[rows], out_hbm.at[rows], sem_out.at[0])

    x_copy(0).start()
    w_copies[0].start()
    for i in range(1, NB):
        x_copy(i).start()
    for cp in w_copies[1:4]:
        cp.start()

    zeros_halo = jnp.zeros((_HALO, D), _F32)
    h_v[pl.ds(0, _HALO), :] = zeros_halo
    h_v[pl.ds(_HALO + S, _HALO), :] = zeros_halo

    def norm_x(i, slot):
        xn = _layernorm(x_v[chunk(i), :].astype(_F32))
        xn_v[chunk(i), :] = xn
        lhs_v[slot] = _layernorm(xn).astype(_BF16)

    x_copy(0).wait()
    norm_x(0, 0)
    w_copies[0].wait()

    def phase1(i, carry):
        @pl.when(i + 1 < NB)
        def _():
            x_copy(i + 1).wait()

        n = D // 2
        h_v[chunk(i, _HALO), :n] = _gelu(_dot(lhs_v[i % 2], weights(w1_v[:, :n])))
        norm_x(jnp.minimum(i + 1, NB - 1), (i + 1) % 2)
        h_v[chunk(i, _HALO), n:] = _gelu(_dot(lhs_v[i % 2], weights(w1_v[:, n:])))
        return carry

    lax.fori_loop(0, NB, phase1, 0)

    w_copies[1].wait()

    def phase2a(i, carry):
        start_group(i)
        c = D // 4
        parts = []
        for q, shift in enumerate((-1, 1, -2, 2)):
            win = h_v[pl.ds(pl.multiple_of(i * TB, TB), TB + 2 * _HALO), q * c:(q + 1) * c]
            parts.append(win[_HALO + shift:_HALO + shift + TB].astype(_BF16))
        hs = _dot(jnp.concatenate(parts, axis=1), weights(w2_v[...]))
        g_v[chunk(i), :] = xn_v[chunk(i), :] + hs
        return carry

    lax.fori_loop(0, NB, phase2a, 0)
    w_copies[4].start()

    def norm_x1(i, slot):
        lhs_v[slot] = _layernorm(g_v[chunk(i), :]).astype(_BF16)

    norm_x1(0, 0)
    w_copies[2].wait()
    w_copies[3].wait()

    def phase2b(i, carry):
        pltpu.make_async_copy(wqkv_v.at[i], wqkv_v.at[i], sem_qkv.at[i]).wait()
        n = F // 2
        ua = _gelu(_dot(lhs_v[i % 2], weights(w3_v[:, :n]))).astype(_BF16)
        norm_x1(jnp.minimum(i + 1, NB - 1), (i + 1) % 2)
        ub = _gelu(_dot(lhs_v[i % 2], weights(w3_v[:, n:]))).astype(_BF16)
        y = g_v[chunk(i), :] + _dot(ua, weights(w4_v[:n // 2, :]))
        g_v[chunk(i), :] = _silu(y + _dot(ub, weights(w4_v[n // 2:, :])))
        repack(i)
        return carry

    lax.fori_loop(0, NB, phase2b, 0)
    w_copies[4].wait()

    row = lax.broadcasted_iota(jnp.int32, (2 * L, DH), 0)
    col = lax.broadcasted_iota(jnp.int32, (2 * L, DH), 1)
    rl = jnp.where(row >= L, row - L, row)
    cl = jnp.where(col >= L, col - L, col)
    same_head = ((row >= L) == (col >= L)) & (col < 2 * L)
    visible = same_head & ((rl < M) | (rl >= cl))
    fill = jnp.where(same_head, -1e9, -jnp.inf).astype(_F32)
    pad = jnp.zeros((DH - 2 * L, DH), _BF16)

    def project(lhs, j):
        c0 = 6 * (j % PG) * DH
        return _dot(lhs, weights(wqkv_v[j // PG, :, c0:c0 + 6 * DH]))

    def pair(r, n):
        return jnp.concatenate(
            [r[:, 2 * n * DH:(2 * n + 1) * DH], r[:, (2 * n + 1) * DH:(2 * n + 2) * DH]],
            axis=0).astype(_BF16)

    def scores(r):
        s = _dot_nt(pair(r, 0), jnp.concatenate([pair(r, 1), pad], axis=0))
        return s, jnp.concatenate([pair(r, 2), pad], axis=0)

    def attend(s, v):
        z = jnp.where(visible, s * scale, fill)
        e = jnp.exp(z - jnp.max(z, axis=-1, keepdims=True))
        p = e / jnp.sum(e, axis=-1, keepdims=True)
        o = _dot(p.astype(_BF16), v)
        return jnp.concatenate([o[:L], o[L:]], axis=1)

    def out_proj(o, j0, j1, n0, n1):
        return _dot(o, weights(wo_v[j0 * DH:j1 * DH, n0:n1]))

    def step(lhs, seq_rows, out_rows):
        LAG = 3
        early = NP - LAG
        nw = D // (LAG + 1)
        rs, sv, os_, ys = {}, {}, [], []
        for j in range(NP + LAG + 1):
            if j < NP:
                rs[j] = seq_rows(j, project(lhs, j))
            else:
                if j == NP:
                    o_early = jnp.concatenate(os_[:early], axis=1)
                ys.append(out_proj(o_early, 0, early, (j - NP) * nw, (j - NP + 1) * nw))
            if 1 <= j <= NP:
                sv[j - 1] = scores(rs.pop(j - 1))
            if LAG <= j < NP + LAG:
                os_.append(out_rows(j - LAG, attend(*sv.pop(j - LAG))).astype(_BF16))
        o_late = jnp.concatenate(os_[early:], axis=1)
        return jnp.concatenate(ys, axis=1) + out_proj(o_late, early, NP, 0, D)

    A = SEG + M
    B = SEG - M

    def phase3(t, mem):
        base = pl.multiple_of(t * 2 * SEG, 2 * SEG)
        held_r, held_o = {}, {}

        def seq_even(j, r):
            held_r[j] = r[L:]
            return r[:L]

        def out_even(j, o):
            held_o[j] = o[M + B:]
            return o[:M + B]

        def seq_odd(j, r):
            return jnp.concatenate([r[:M], held_r[j], r[M:]], axis=0)

        def out_odd(j, o):
            return jnp.concatenate([o[:M], held_o[j], o[M:]], axis=0)

        lhs0 = jnp.concatenate([mem, xn_v[pl.ds(base, A), :]], axis=0).astype(_BF16)
        y0 = step(lhs0, seq_even, out_even)
        rest = pl.ds(pl.multiple_of(base + A, 8), 2 * SEG - A)
        lhs1 = jnp.concatenate([y0[:M], xn_v[rest, :]], axis=0).astype(_BF16)
        y1 = step(lhs1, seq_odd, out_odd)

        rows = pl.ds(base, 2 * SEG)
        s = jnp.concatenate([y0[M:], y1[M:]], axis=0)
        o_v[rows, :] = (x_v[rows, :].astype(_F32) + s * g_v[rows, :]).astype(o_v.dtype)
        out_copy(t).start()
        return y1[:M]

    lax.fori_loop(0, S // (2 * SEG), phase3, mem0_ref[...].astype(_F32))
    pltpu.make_async_copy(o_v, out_hbm, sem_out.at[0]).wait()


@functools.partial(jax.jit, static_argnames=("A_seg_len",))
def pallas_recurrent_scan__memory_aug_recurrent_mem_tr__mixer_s_mlp__prompt_kernel(
    A_x: jax.Array,
    A_mem0: jax.Array,
    A_Wq: jax.Array,
    A_Wk: jax.Array,
    A_Wv: jax.Array,
    A_Wo: jax.Array,
    A_seg_len: int,
    B_x: jax.Array,
    B_w1: jax.Array,
    B_w2: jax.Array,
    B_w3: jax.Array,
    B_w4: jax.Array,
):
    del B_x
    batch, S, D = A_x.shape
    _, H, DH = A_Wq.shape
    M = A_mem0.shape[1]
    F = B_w3.shape[1]
    SEG = int(A_seg_len)
    TB = 256
    NB = S // TB
    assert batch == 1 and DH == 128 and M == 8 and SEG % 16 == 0 and 2 * (M + SEG) <= DH
    assert S % TB == 0 and S % (2 * SEG) == 0 and D % (16 * NB) == 0 and H % 2 == 0
    out_dtype = A_x.dtype

    hbm = pl.BlockSpec(memory_space=pl.ANY)
    out = pl.pallas_call(
        functools.partial(_kernel, S=S, D=D, H=H, DH=DH, F=F, M=M, SEG=SEG, TB=TB),
        out_shape=jax.ShapeDtypeStruct((S, D), out_dtype),
        in_specs=[hbm, pl.BlockSpec(memory_space=pltpu.VMEM)] + [hbm] * 8,
        out_specs=hbm,
        scratch_shapes=[
            pltpu.VMEM((S, D), _BF16),
            pltpu.VMEM((S, D), out_dtype),
            pltpu.VMEM((S, D), _F32),
            pltpu.VMEM((S + 2 * _HALO, D), _F32),
            pltpu.VMEM((S, D), _F32),
            pltpu.VMEM((2, TB, D), _BF16),
            pltpu.VMEM((D // 2, D), _U32),
            pltpu.VMEM((D // 2, D), _U32),
            pltpu.VMEM((D // 2, F), _U32),
            pltpu.VMEM((F // 2, D), _U32),
            pltpu.VMEM((NB, D // 2, 3 * H * DH // NB), _U32),
            pltpu.VMEM((H * DH // 2, D), _U32),
            pltpu.SemaphoreType.DMA((NB,)),
            pltpu.SemaphoreType.DMA((5,)),
            pltpu.SemaphoreType.DMA((NB,)),
            pltpu.SemaphoreType.DMA((1,)),
        ],
        compiler_params=pltpu.CompilerParams(vmem_limit_bytes=120 * 1024 * 1024),
    )(
        A_x.reshape(S, D),
        A_mem0.reshape(M, D),
        A_Wq.reshape(D // 2, 2, H, DH),
        A_Wk.reshape(D // 2, 2, H, DH),
        A_Wv.reshape(D // 2, 2, H, DH),
        A_Wo.reshape(H * DH, D),
        B_w1, B_w2, B_w3, B_w4,
    )
    return out.reshape(batch, S, D)
```

```python
import functools

import jax
import jax.numpy as jnp
from jax import lax
import jax.experimental.pallas as pl
import jax.experimental.pallas.tpu as pltpu

_EPS = 1e-5
_HALO = 8
_F32 = jnp.float32
_BF16 = jnp.bfloat16
_U32 = jnp.uint32


def _layernorm(v):
    m = jnp.mean(v, axis=-1, keepdims=True)
    c = v - m
    var = jnp.mean(c * c, axis=-1, keepdims=True)
    return c * lax.rsqrt(var + _EPS)


def _gelu(v):
    c = 0.7978845608028654
    h = 0.5 * v
    return h + h * jnp.tanh(v * (c + (c * 0.044715) * (v * v)))


def _silu(v):
    h = 0.5 * v
    return h + h * jnp.tanh(h)


def _dot(a, b):
    return jnp.dot(a, b, preferred_element_type=_F32)


def _dot_nt(a, b):
    return lax.dot_general(a, b, (((1,), (1,)), ((), ())), preferred_element_type=_F32)


def _strassen_lhs(a11, a12, a21, a22):
    sums = (a11 + a22, a21 + a22, a11, a22, a11 + a12, a21 - a11, a12 - a22)
    return [t.astype(_BF16) for t in sums]


def _strassen_dot(product):
    m5 = product(4)
    m3 = product(2)
    c12 = m3 + m5
    m4 = product(3)
    m2 = product(1)
    c21 = m2 + m4
    c11 = m4 - m5 + product(6)
    c22 = m3 - m2 + product(5)
    m1 = product(0)
    return c11 + m1, c12, c21, c22 + m1


def _kernel(
    x_hbm, mem0_ref, wq_hbm, wk_hbm, wv_hbm, wo_hbm, w1_hbm, w2_hbm, w3_hbm, w4_hbm,
    out_hbm,
    x_v, o_v, xn_v, h_v, g_v, lhs_v, ls_v, w1_v, w2_v, w3_v, w4_v, e3_v, e4_v,
    wqkv_v, wo_v,
    sem_x, sem_w, sem_qkv, sem_out,
    *, S, D, H, DH, F, M, SEG, TB,
):
    NB = S // TB
    NP = H // 2
    PG = NP // NB
    L = M + SEG
    scale = DH ** (-0.5)

    def weights(ref):
        return pltpu.bitcast(ref, _BF16)

    def chunk(i, offset=0):
        return pl.ds(pl.multiple_of(i * TB + offset, 8), TB)

    def x_copy(i):
        rows = pl.ds(pl.multiple_of(i * TB, TB), TB)
        return pltpu.make_async_copy(x_hbm.at[rows], x_v.at[rows], sem_x.at[i])

    w_copies = [
        pltpu.make_async_copy(src, dst.bitcast(_BF16), sem_w.at[n])
        for n, (src, dst) in enumerate(
            ((w1_hbm, w1_v), (w2_hbm, w2_v), (w3_hbm, w3_v), (w4_hbm, w4_v), (wo_hbm, wo_v)))
    ]

    def start_group(i):
        for n, w in enumerate((wq_hbm, wk_hbm, wv_hbm)):
            w32 = w.bitcast(_U32)
            for p in range(PG):
                for parity in range(2):
                    c0 = (6 * p + 2 * n + parity) * DH
                    pltpu.make_async_copy(
                        w32.at[:, parity, i * PG + p, :],
                        wqkv_v.at[i, :, pl.ds(c0, DH)],
                        sem_qkv.at[i]).start()

    def repack(i):
        for c0 in range(0, 6 * PG * DH, 2 * DH):
            for r0 in range(0, D // 2, 8):
                rows = slice(r0, r0 + 8)
                ev = wqkv_v[i, rows, c0:c0 + DH]
                od = wqkv_v[i, rows, c0 + DH:c0 + 2 * DH]
                wqkv_v[i, rows, c0:c0 + DH] = (ev & _U32(0xFFFF)) | (od << 16)
                wqkv_v[i, rows, c0 + DH:c0 + 2 * DH] = (ev >> 16) | (od & _U32(0xFFFF0000))

    def out_copy(t):
        rows = pl.ds(pl.multiple_of(t * 2 * SEG, 2 * SEG), 2 * SEG)
        return pltpu.make_async_copy(o_v.at[rows], out_hbm.at[rows], sem_out.at[0])

    x_copy(0).start()
    w_copies[0].start()
    for i in range(1, NB):
        x_copy(i).start()
    for cp in w_copies[1:4]:
        cp.start()

    zeros_halo = jnp.zeros((_HALO, D), _F32)
    h_v[pl.ds(0, _HALO), :] = zeros_halo
    h_v[pl.ds(_HALO + S, _HALO), :] = zeros_halo

    def norm_x(i, slot, r0=0, r1=TB):
        rows = pl.ds(pl.multiple_of(i * TB + r0, 16), r1 - r0)
        xn = _layernorm(x_v[rows, :].astype(_F32))
        xn_v[rows, :] = xn
        lhs_v[slot, r0:r1, :] = _layernorm(xn).astype(_BF16)

    x_copy(0).wait()
    norm_x(0, 0)
    w_copies[0].wait()

    def phase1(i, carry):
        @pl.when(i + 1 < NB)
        def _():
            x_copy(i + 1).wait()

        n = D // 4
        cuts = (0, 80, 176, 256)
        for q in range(4):
            h_v[chunk(i, _HALO), q * n:(q + 1) * n] = _gelu(_dot(lhs_v[i % 2], weights(w1_v[:, q * n:(q + 1) * n])))
            if q < 4 - 1:
                norm_x(jnp.minimum(i + 1, NB - 1), (i + 1) % 2, cuts[q], cuts[q + 1])
        return carry

    lax.fori_loop(0, NB, phase1, 0)

    def block_sum_jobs(i):
        for w_v, e_v in ((w3_v, e3_v), (w4_v, e4_v)):
            kh, nh = w_v.shape[0] // 2, w_v.shape[1] // 2
            nr = kh // NB
            for r in range(0, nr, 8):
                top = pl.ds(pl.multiple_of(i * nr + r, 8), 8)
                bot = pl.ds(pl.multiple_of(kh + i * nr + r, 8), 8)
                for c in range(0, nh, 128):
                    yield w_v, e_v, top, bot, slice(c, c + 128), slice(nh + c, nh + c + 128)

    def block_sums(jobs, dep, zero):
        for w_v, e_v, top, bot, left, right in jobs:
            d = dep & zero
            b11, b12 = weights(w_v[top, left] | d), weights(w_v[top, right])
            b21, b22 = weights(w_v[bot, left]), weights(w_v[bot, right] | d)
            e_v[0, top, left] = pltpu.bitcast(b11 + b22, _U32)
            e_v[1, top, left] = pltpu.bitcast(b11 + b12, _U32)
            e_v[2, top, left] = pltpu.bitcast(b21 + b22, _U32)
            w_v[top, right] = pltpu.bitcast(b12 - b22, _U32)
            t4 = pltpu.bitcast(b21 - b11, _U32)
            w_v[bot, left] = t4
            if True:
                dep = t4

    def strassen_rhs(w_v, e_v, k, r0, r1, c0, c1):
        kh, nh = w_v.shape[0] // 2, w_v.shape[1] // 2
        r0, r1 = r0 // 2, r1 // 2
        if k in (0, 5, 6):
            return weights(e_v[{0: 0, 5: 1, 6: 2}[k], r0:r1, c0:c1])
        dr, dc = {1: (0, 0), 2: (0, nh), 3: (kh, 0), 4: (kh, nh)}[k]
        return weights(w_v[dr + r0:dr + r1, dc + c0:dc + c1])

    for cp in w_copies[1:4]:
        cp.wait()

    def phase2a(i, carry):
        start_group(i)
        c = D // 4
        parts = []
        for q, shift in enumerate((-1, 1, -2, 2)):
            win = h_v[pl.ds(pl.multiple_of(i * TB, TB), TB + 2 * _HALO), q * c:(q + 1) * c]
            parts.append(win[_HALO + shift:_HALO + shift + TB].astype(_BF16))
        lhs = jnp.concatenate(parts, axis=1)
        zero = pltpu.bitcast(h_v[0:8, 0:128], _U32)
        jobs = list(block_sum_jobs(i))
        n = D // 8
        for q in range(8):
            cols = slice(q * n, (q + 1) * n)
            x1 = xn_v[chunk(i), cols] + _dot(lhs, weights(w2_v[:, cols]))
            g_v[chunk(i), cols] = x1
            if q < 8 - 1:
                part = jobs[q * len(jobs) // (8 - 1):(q + 1) * len(jobs) // (8 - 1)]
                block_sums(part, pltpu.bitcast(x1[:8, :128], _U32), zero)
        return carry

    lax.fori_loop(0, NB, phase2a, 0)
    w_copies[4].start()

    HB, DHALF, FHALF = TB // 2, D // 2, F // 2

    def half(i, k, r0=0, r1=HB):
        return pl.ds(pl.multiple_of(i * TB + k * HB + r0, 16), r1 - r0)

    def norm_x1(i, slot, r0=0, r1=HB):
        top = _layernorm(g_v[half(i, 0, r0, r1), :])
        bot = _layernorm(g_v[half(i, 1, r0, r1), :])
        ops = _strassen_lhs(top[:, :DHALF], top[:, DHALF:], bot[:, :DHALF], bot[:, DHALF:])
        for k in range(7):
            ls_v[slot, k, r0:r1, :] = ops[k]

    norm_x1(0, 0)

    def phase2b(i, carry):
        pltpu.make_async_copy(wqkv_v.at[i], wqkv_v.at[i], sem_qkv.at[i]).wait()
        us = []
        for n, c0 in enumerate(range(0, FHALF, 256)):
            pre = _strassen_dot(lambda k: _dot(
                ls_v[i % 2, k], strassen_rhs(w3_v, e3_v, k, 0, DHALF, c0, c0 + 256)))
            us.append(_strassen_lhs(*[_gelu(t) for t in pre]))
            m = n * 256 // 256
            if (n * 256) % 256 == 0 and m < 4:
                norm_x1(jnp.minimum(i + 1, NB - 1), (i + 1) % 2, m * HB // 4, (m + 1) * HB // 4)
        u = [jnp.concatenate([t[k] for t in us], axis=1) for k in range(7)]
        cut = FHALF - 512
        first = (0, 256, 384, 512)[1]
        head = {k: _dot(u[k][:, :cut], strassen_rhs(w4_v, e4_v, k, 0, cut, 0, first))
                for k in (4, 2, 3)}
        for c0, c1 in zip((0, 256, 384, 512)[:-1], (0, 256, 384, 512)[1:]):
            def product(k):
                if k in head:
                    return head.pop(k) + _dot(
                        u[k][:, cut:], strassen_rhs(w4_v, e4_v, k, cut, FHALF, c0, c1))
                return _dot(u[k], strassen_rhs(w4_v, e4_v, k, 0, FHALF, c0, c1))
            for n, y in enumerate(_strassen_dot(product)):
                rows = half(i, n // 2)
                cols = slice((n % 2) * DHALF + c0, (n % 2) * DHALF + c1)
                g_v[rows, cols] = _silu(g_v[rows, cols] + y)
        repack(i)
        return carry

    lax.fori_loop(0, NB, phase2b, 0)
    w_copies[4].wait()

    row = lax.broadcasted_iota(jnp.int32, (2 * L, DH), 0)
    col = lax.broadcasted_iota(jnp.int32, (2 * L, DH), 1)
    rl = jnp.where(row >= L, row - L, row)
    cl = jnp.where(col >= L, col - L, col)
    same_head = ((row >= L) == (col >= L)) & (col < 2 * L)
    visible = same_head & ((rl < M) | (rl >= cl))
    fill = jnp.where(same_head, -1e9, -jnp.inf).astype(_F32)
    pad = jnp.zeros((DH - 2 * L, DH), _BF16)

    def project(lhs, j):
        c0 = 6 * (j % PG) * DH
        return _dot(lhs, weights(wqkv_v[j // PG, :, c0:c0 + 6 * DH]))

    def pair(r, n):
        return jnp.concatenate(
            [r[:, 2 * n * DH:(2 * n + 1) * DH], r[:, (2 * n + 1) * DH:(2 * n + 2) * DH]],
            axis=0).astype(_BF16)

    def scores(r):
        s = _dot_nt(pair(r, 0), jnp.concatenate([pair(r, 1), pad], axis=0))
        return s, jnp.concatenate([pair(r, 2), pad], axis=0)

    def attend(s, v):
        z = jnp.where(visible, s * scale, fill)
        e = jnp.exp(z - jnp.max(z, axis=-1, keepdims=True))
        p = e / jnp.sum(e, axis=-1, keepdims=True)
        o = _dot(p.astype(_BF16), v)
        return jnp.concatenate([o[:L], o[L:]], axis=1)

    def out_proj(o, j0, j1, n0, n1):
        return _dot(o, weights(wo_v[j0 * DH:j1 * DH, n0:n1]))

    def step(lhs, seq_rows, out_rows):
        LAG = 3
        early = NP - LAG
        nw = D // (LAG + 1)
        rs, sv, os_, ys = {}, {}, [], []
        for j in range(NP + LAG + 1):
            if j < NP:
                rs[j] = seq_rows(j, project(lhs, j))
            else:
                if j == NP:
                    o_early = jnp.concatenate(os_[:early], axis=1)
                ys.append(out_proj(o_early, 0, early, (j - NP) * nw, (j - NP + 1) * nw))
            if 1 <= j <= NP:
                sv[j - 1] = scores(rs.pop(j - 1))
            if LAG <= j < NP + LAG:
                os_.append(out_rows(j - LAG, attend(*sv.pop(j - LAG))).astype(_BF16))
        o_late = jnp.concatenate(os_[early:], axis=1)
        return jnp.concatenate(ys, axis=1) + out_proj(o_late, early, NP, 0, D)

    A = SEG + M
    B = SEG - M

    def phase3(t, mem):
        base = pl.multiple_of(t * 2 * SEG, 2 * SEG)
        held_r, held_o = {}, {}

        def seq_even(j, r):
            held_r[j] = r[L:]
            return r[:L]

        def out_even(j, o):
            held_o[j] = o[M + B:]
            return o[:M + B]

        def seq_odd(j, r):
            return jnp.concatenate([r[:M], held_r[j], r[M:]], axis=0)

        def out_odd(j, o):
            return jnp.concatenate([o[:M], held_o[j], o[M:]], axis=0)

        lhs0 = jnp.concatenate([mem, xn_v[pl.ds(base, A), :]], axis=0).astype(_BF16)
        y0 = step(lhs0, seq_even, out_even)
        rest = pl.ds(pl.multiple_of(base + A, 8), 2 * SEG - A)
        lhs1 = jnp.concatenate([y0[:M], xn_v[rest, :]], axis=0).astype(_BF16)
        y1 = step(lhs1, seq_odd, out_odd)

        rows = pl.ds(base, 2 * SEG)
        s = jnp.concatenate([y0[M:], y1[M:]], axis=0)
        o_v[rows, :] = (x_v[rows, :].astype(_F32) + s * g_v[rows, :]).astype(o_v.dtype)
        out_copy(t).start()
        return y1[:M]

    lax.fori_loop(0, S // (2 * SEG), phase3, mem0_ref[...].astype(_F32))
    pltpu.make_async_copy(o_v, out_hbm, sem_out.at[0]).wait()


@functools.partial(jax.jit, static_argnames=("A_seg_len",))
def pallas_recurrent_scan__memory_aug_recurrent_mem_tr__mixer_s_mlp__prompt_kernel(
    A_x: jax.Array,
    A_mem0: jax.Array,
    A_Wq: jax.Array,
    A_Wk: jax.Array,
    A_Wv: jax.Array,
    A_Wo: jax.Array,
    A_seg_len: int,
    B_x: jax.Array,
    B_w1: jax.Array,
    B_w2: jax.Array,
    B_w3: jax.Array,
    B_w4: jax.Array,
):
    del B_x
    batch, S, D = A_x.shape
    _, H, DH = A_Wq.shape
    M = A_mem0.shape[1]
    F = B_w3.shape[1]
    SEG = int(A_seg_len)
    TB = 256
    NB = S // TB
    assert batch == 1 and DH == 128 and M == 8 and SEG % 16 == 0 and 2 * (M + SEG) <= DH
    assert S % TB == 0 and S % (2 * SEG) == 0 and D % (16 * NB) == 0 and H % 2 == 0
    out_dtype = A_x.dtype

    hbm = pl.BlockSpec(memory_space=pl.ANY)
    out = pl.pallas_call(
        functools.partial(_kernel, S=S, D=D, H=H, DH=DH, F=F, M=M, SEG=SEG, TB=TB),
        out_shape=jax.ShapeDtypeStruct((S, D), out_dtype),
        in_specs=[hbm, pl.BlockSpec(memory_space=pltpu.VMEM)] + [hbm] * 8,
        out_specs=hbm,
        scratch_shapes=[
            pltpu.VMEM((S, D), _BF16),
            pltpu.VMEM((S, D), out_dtype),
            pltpu.VMEM((S, D), _F32),
            pltpu.VMEM((S + 2 * _HALO, D), _F32),
            pltpu.VMEM((S, D), _F32),
            pltpu.VMEM((2, TB, D), _BF16),
            pltpu.VMEM((2, 7, TB // 2, D // 2), _BF16),
            pltpu.VMEM((D // 2, D), _U32),
            pltpu.VMEM((D // 2, D), _U32),
            pltpu.VMEM((D // 2, F), _U32),
            pltpu.VMEM((F // 2, D), _U32),
            pltpu.VMEM((3, D // 4, F // 2), _U32),
            pltpu.VMEM((3, F // 4, D // 2), _U32),
            pltpu.VMEM((NB, D // 2, 3 * H * DH // NB), _U32),
            pltpu.VMEM((H * DH // 2, D), _U32),
            pltpu.SemaphoreType.DMA((NB,)),
            pltpu.SemaphoreType.DMA((5,)),
            pltpu.SemaphoreType.DMA((NB,)),
            pltpu.SemaphoreType.DMA((1,)),
        ],
        compiler_params=pltpu.CompilerParams(vmem_limit_bytes=120 * 1024 * 1024),
    )(
        A_x.reshape(S, D),
        A_mem0.reshape(M, D),
        A_Wq.reshape(D // 2, 2, H, DH),
        A_Wk.reshape(D // 2, 2, H, DH),
        A_Wv.reshape(D // 2, 2, H, DH),
        A_Wo.reshape(H * DH, D),
        B_w1, B_w2, B_w3, B_w4,
    )
    return out.reshape(batch, S, D)
```

```python
import functools

import jax
import jax.numpy as jnp
from jax import lax
import jax.experimental.pallas as pl
import jax.experimental.pallas.tpu as pltpu

_EPS = 1e-5
_HALO = 8
_F32 = jnp.float32
_BF16 = jnp.bfloat16
_U32 = jnp.uint32


def _layernorm(v):
    m = jnp.mean(v, axis=-1, keepdims=True)
    c = v - m
    var = jnp.mean(c * c, axis=-1, keepdims=True)
    return c * lax.rsqrt(var + _EPS)


def _gelu(v):
    c = 0.7978845608028654
    h = 0.5 * v
    return h + h * jnp.tanh(v * (c + (c * 0.044715) * (v * v)))


def _silu(v):
    h = 0.5 * v
    return h + h * jnp.tanh(h)


def _dot(a, b):
    return jnp.dot(a, b, preferred_element_type=_F32)


def _dot_nt(a, b):
    return lax.dot_general(a, b, (((1,), (1,)), ((), ())), preferred_element_type=_F32)


def _strassen_lhs(a11, a12, a21, a22):
    sums = (a11 + a22, a21 + a22, a11, a22, a11 + a12, a21 - a11, a12 - a22)
    return [t.astype(_BF16) for t in sums]


def _strassen_dot(product):
    m5 = product(4)
    m3 = product(2)
    c12 = m3 + m5
    m4 = product(3)
    m2 = product(1)
    c21 = m2 + m4
    c11 = m4 - m5 + product(6)
    c22 = m3 - m2 + product(5)
    m1 = product(0)
    return c11 + m1, c12, c21, c22 + m1


def _kernel(
    x_hbm, mem0_ref, wq_hbm, wk_hbm, wv_hbm, wo_hbm, w1_hbm, w2_hbm, w3_hbm, w4_hbm,
    out_hbm,
    x_v, o_v, xn_v, h_v, g_v, lhs_v, ls_v, w1_v, w2_v, w3_v, w4_v, e3_v, e4_v,
    wqkv_v, wo_v,
    sem_x, sem_w, sem_qkv, sem_out,
    *, S, D, H, DH, F, M, SEG, TB,
):
    NB = S // TB
    NP = H // 2
    PG = NP // NB
    L = M + SEG
    scale = DH ** (-0.5)

    def weights(ref):
        return pltpu.bitcast(ref, _BF16)

    def chunk(i, offset=0):
        return pl.ds(pl.multiple_of(i * TB + offset, 8), TB)

    def x_copy(i):
        rows = pl.ds(pl.multiple_of(i * TB, TB), TB)
        return pltpu.make_async_copy(x_hbm.at[rows], x_v.at[rows], sem_x.at[i])

    w_copies = [
        pltpu.make_async_copy(src, dst.bitcast(_BF16), sem_w.at[n])
        for n, (src, dst) in enumerate(
            ((w1_hbm, w1_v), (w2_hbm, w2_v), (w3_hbm, w3_v), (w4_hbm, w4_v), (wo_hbm, wo_v)))
    ]

    def start_group(i):
        for n, w in enumerate((wq_hbm, wk_hbm, wv_hbm)):
            w32 = w.bitcast(_U32)
            for p in range(PG):
                for parity in range(2):
                    c0 = (6 * p + 2 * n + parity) * DH
                    pltpu.make_async_copy(
                        w32.at[:, parity, i * PG + p, :],
                        wqkv_v.at[i, :, pl.ds(c0, DH)],
                        sem_qkv.at[i]).start()

    def repack(i):
        for c0 in range(0, 6 * PG * DH, 2 * DH):
            for r0 in range(0, D // 2, 8):
                rows = slice(r0, r0 + 8)
                ev = wqkv_v[i, rows, c0:c0 + DH]
                od = wqkv_v[i, rows, c0 + DH:c0 + 2 * DH]
                wqkv_v[i, rows, c0:c0 + DH] = (ev & _U32(0xFFFF)) | (od << 16)
                wqkv_v[i, rows, c0 + DH:c0 + 2 * DH] = (ev >> 16) | (od & _U32(0xFFFF0000))

    def out_copy(t):
        rows = pl.ds(pl.multiple_of(t * 2 * SEG, 2 * SEG), 2 * SEG)
        return pltpu.make_async_copy(o_v.at[rows], out_hbm.at[rows], sem_out.at[0])

    x_copy(0).start()
    w_copies[0].start()
    for i in range(1, NB):
        x_copy(i).start()
    for cp in w_copies[1:4]:
        cp.start()

    zeros_halo = jnp.zeros((_HALO, D), _F32)
    h_v[pl.ds(0, _HALO), :] = zeros_halo
    h_v[pl.ds(_HALO + S, _HALO), :] = zeros_halo

    def norm_x(i, slot, r0=0, r1=TB):
        rows = pl.ds(pl.multiple_of(i * TB + r0, 16), r1 - r0)
        xn = _layernorm(x_v[rows, :].astype(_F32))
        xn_v[rows, :] = xn
        lhs_v[slot, r0:r1, :] = _layernorm(xn).astype(_BF16)

    x_copy(0).wait()
    norm_x(0, 0)
    w_copies[0].wait()

    def phase1(i, carry):
        @pl.when(i + 1 < NB)
        def _():
            x_copy(i + 1).wait()

        n = D // 4
        cuts = (0, 80, 176, 256)
        for q in range(4):
            h_v[chunk(i, _HALO), q * n:(q + 1) * n] = _gelu(_dot(lhs_v[i % 2], weights(w1_v[:, q * n:(q + 1) * n])))
            if q < 4 - 1:
                norm_x(jnp.minimum(i + 1, NB - 1), (i + 1) % 2, cuts[q], cuts[q + 1])
        return carry

    lax.fori_loop(0, NB, phase1, 0)

    def block_sum_jobs(w_v, i, parts):
        kh, nh = w_v.shape[0] // 2, w_v.shape[1] // 2
        nr = kh // parts
        for r in range(0, nr, 8):
            top = pl.ds(pl.multiple_of(i * nr + r, 8), 8)
            bot = pl.ds(pl.multiple_of(kh + i * nr + r, 8), 8)
            for c in range(0, nh, 128):
                yield top, bot, slice(c, c + 128), slice(nh + c, nh + c + 128)

    def block_sums(w_v, e_v, jobs, dep, zero):
        for top, bot, left, right in jobs:
            d = dep & zero
            b11, b12 = weights(w_v[top, left] | d), weights(w_v[top, right])
            b21, b22 = weights(w_v[bot, left]), weights(w_v[bot, right] | d)
            e_v[0, top, left] = pltpu.bitcast(b11 + b22, _U32)
            e_v[1, top, left] = pltpu.bitcast(b11 + b12, _U32)
            e_v[2, top, left] = pltpu.bitcast(b21 + b22, _U32)
            w_v[top, right] = pltpu.bitcast(b12 - b22, _U32)
            dep = pltpu.bitcast(b21 - b11, _U32)
            w_v[bot, left] = dep

    def strassen_rhs(w_v, e_v, k, r0, r1, c0, c1):
        kh, nh = w_v.shape[0] // 2, w_v.shape[1] // 2
        r0, r1 = r0 // 2, r1 // 2
        if k in (0, 5, 6):
            return weights(e_v[{0: 0, 5: 1, 6: 2}[k], r0:r1, c0:c1])
        dr, dc = {1: (0, 0), 2: (0, nh), 3: (kh, 0), 4: (kh, nh)}[k]
        return weights(w_v[dr + r0:dr + r1, dc + c0:dc + c1])

    def phase2a(w_v, e_v, first, i, carry):
        start_group(i)
        c = D // 4
        parts = []
        for q, shift in enumerate((-1, 1, -2, 2)):
            win = h_v[pl.ds(pl.multiple_of(i * TB, TB), TB + 2 * _HALO), q * c:(q + 1) * c]
            parts.append(win[_HALO + shift:_HALO + shift + TB].astype(_BF16))
        lhs = jnp.concatenate(parts, axis=1)
        zero = pltpu.bitcast(h_v[0:8, 0:128], _U32)
        jobs = list(block_sum_jobs(w_v, i - first, NB // 2))
        n = D // 8
        for q in range(8):
            cols = slice(q * n, (q + 1) * n)
            x1 = xn_v[chunk(i), cols] + _dot(lhs, weights(w2_v[:, cols]))
            g_v[chunk(i), cols] = x1
            if q < 8 - 1:
                part = jobs[q * len(jobs) // (8 - 1):(q + 1) * len(jobs) // (8 - 1)]
                block_sums(w_v, e_v, part, pltpu.bitcast(x1[:8, :128], _U32), zero)
        return carry

    w_copies[1].wait()
    w_copies[2].wait()
    lax.fori_loop(0, NB // 2, functools.partial(phase2a, w3_v, e3_v, 0), 0)
    w_copies[3].wait()
    lax.fori_loop(NB // 2, NB, functools.partial(phase2a, w4_v, e4_v, NB // 2), 0)
    w_copies[4].start()

    HB, DHALF, FHALF = TB // 2, D // 2, F // 2

    def half(i, k, r0=0, r1=HB):
        return pl.ds(pl.multiple_of(i * TB + k * HB + r0, 16), r1 - r0)

    def norm_x1(i, slot, r0=0, r1=HB):
        top = _layernorm(g_v[half(i, 0, r0, r1), :])
        bot = _layernorm(g_v[half(i, 1, r0, r1), :])
        ops = _strassen_lhs(top[:, :DHALF], top[:, DHALF:], bot[:, :DHALF], bot[:, DHALF:])
        for k in range(7):
            ls_v[slot, k, r0:r1, :] = ops[k]

    norm_x1(0, 0)

    def phase2b(i, carry):
        pltpu.make_async_copy(wqkv_v.at[i], wqkv_v.at[i], sem_qkv.at[i]).wait()
        us = []
        for n, c0 in enumerate(range(0, FHALF, 256)):
            pre = _strassen_dot(lambda k: _dot(
                ls_v[i % 2, k], strassen_rhs(w3_v, e3_v, k, 0, DHALF, c0, c0 + 256)))
            us.append(_strassen_lhs(*[_gelu(t) for t in pre]))
            m = n * 256 // 256
            if (n * 256) % 256 == 0 and m < 4:
                norm_x1(jnp.minimum(i + 1, NB - 1), (i + 1) % 2, m * HB // 4, (m + 1) * HB // 4)
        u = [jnp.concatenate([t[k] for t in us], axis=1) for k in range(7)]
        cut = FHALF - 512
        first = (0, 256, 384, 512)[1]
        head = {k: _dot(u[k][:, :cut], strassen_rhs(w4_v, e4_v, k, 0, cut, 0, first))
                for k in (4, 2, 3)}
        for c0, c1 in zip((0, 256, 384, 512)[:-1], (0, 256, 384, 512)[1:]):
            def product(k):
                if k in head:
                    return head.pop(k) + _dot(
                        u[k][:, cut:], strassen_rhs(w4_v, e4_v, k, cut, FHALF, c0, c1))
                return _dot(u[k], strassen_rhs(w4_v, e4_v, k, 0, FHALF, c0, c1))
            for n, y in enumerate(_strassen_dot(product)):
                rows = half(i, n // 2)
                cols = slice((n % 2) * DHALF + c0, (n % 2) * DHALF + c1)
                g_v[rows, cols] = _silu(g_v[rows, cols] + y)
        repack(i)
        return carry

    lax.fori_loop(0, NB, phase2b, 0)
    w_copies[4].wait()

    row = lax.broadcasted_iota(jnp.int32, (2 * L, DH), 0)
    col = lax.broadcasted_iota(jnp.int32, (2 * L, DH), 1)
    rl = jnp.where(row >= L, row - L, row)
    cl = jnp.where(col >= L, col - L, col)
    same_head = ((row >= L) == (col >= L)) & (col < 2 * L)
    visible = same_head & ((rl < M) | (rl >= cl))
    fill = jnp.where(same_head, -1e9, -jnp.inf).astype(_F32)
    pad = jnp.zeros((DH - 2 * L, DH), _BF16)

    def project(lhs, j):
        c0 = 6 * (j % PG) * DH
        return _dot(lhs, weights(wqkv_v[j // PG, :, c0:c0 + 6 * DH]))

    def pair(r, n):
        return jnp.concatenate(
            [r[:, 2 * n * DH:(2 * n + 1) * DH], r[:, (2 * n + 1) * DH:(2 * n + 2) * DH]],
            axis=0).astype(_BF16)

    def scores(r):
        s = _dot_nt(pair(r, 0), jnp.concatenate([pair(r, 1), pad], axis=0))
        return s, jnp.concatenate([pair(r, 2), pad], axis=0)

    def attend(s, v):
        z = jnp.where(visible, s * scale, fill)
        e = jnp.exp(z - jnp.max(z, axis=-1, keepdims=True))
        p = e / jnp.sum(e, axis=-1, keepdims=True)
        o = _dot(p.astype(_BF16), v)
        return jnp.concatenate([o[:L], o[L:]], axis=1)

    def out_proj(o, j0, j1, n0, n1):
        return _dot(o, weights(wo_v[j0 * DH:j1 * DH, n0:n1]))

    def step(lhs, seq_rows, out_rows):
        LAG = 3
        early = NP - LAG
        nw = D // (LAG + 1)
        rs, sv, os_, ys = {}, {}, [], []
        for j in range(NP + LAG + 1):
            if j < NP:
                rs[j] = seq_rows(j, project(lhs, j))
            else:
                if j == NP:
                    o_early = jnp.concatenate(os_[:early], axis=1)
                ys.append(out_proj(o_early, 0, early, (j - NP) * nw, (j - NP + 1) * nw))
            if 1 <= j <= NP:
                sv[j - 1] = scores(rs.pop(j - 1))
            if LAG <= j < NP + LAG:
                os_.append(out_rows(j - LAG, attend(*sv.pop(j - LAG))).astype(_BF16))
        o_late = jnp.concatenate(os_[early:], axis=1)
        return jnp.concatenate(ys, axis=1) + out_proj(o_late, early, NP, 0, D)

    A = SEG + M
    B = SEG - M

    def phase3(t, mem):
        base = pl.multiple_of(t * 2 * SEG, 2 * SEG)
        held_r, held_o = {}, {}

        def seq_even(j, r):
            held_r[j] = r[L:]
            return r[:L]

        def out_even(j, o):
            held_o[j] = o[M + B:]
            return o[:M + B]

        def seq_odd(j, r):
            return jnp.concatenate([r[:M], held_r[j], r[M:]], axis=0)

        def out_odd(j, o):
            return jnp.concatenate([o[:M], held_o[j], o[M:]], axis=0)

        lhs0 = jnp.concatenate([mem, xn_v[pl.ds(base, A), :]], axis=0).astype(_BF16)
        y0 = step(lhs0, seq_even, out_even)
        rest = pl.ds(pl.multiple_of(base + A, 8), 2 * SEG - A)
        lhs1 = jnp.concatenate([y0[:M], xn_v[rest, :]], axis=0).astype(_BF16)
        y1 = step(lhs1, seq_odd, out_odd)

        rows = pl.ds(base, 2 * SEG)
        s = jnp.concatenate([y0[M:], y1[M:]], axis=0)
        o_v[rows, :] = (x_v[rows, :].astype(_F32) + s * g_v[rows, :]).astype(o_v.dtype)
        out_copy(t).start()
        return y1[:M]

    lax.fori_loop(0, S // (2 * SEG), phase3, mem0_ref[...].astype(_F32))
    pltpu.make_async_copy(o_v, out_hbm, sem_out.at[0]).wait()


@functools.partial(jax.jit, static_argnames=("A_seg_len",))
def pallas_recurrent_scan__memory_aug_recurrent_mem_tr__mixer_s_mlp__prompt_kernel(
    A_x: jax.Array,
    A_mem0: jax.Array,
    A_Wq: jax.Array,
    A_Wk: jax.Array,
    A_Wv: jax.Array,
    A_Wo: jax.Array,
    A_seg_len: int,
    B_x: jax.Array,
    B_w1: jax.Array,
    B_w2: jax.Array,
    B_w3: jax.Array,
    B_w4: jax.Array,
):
    del B_x
    batch, S, D = A_x.shape
    _, H, DH = A_Wq.shape
    M = A_mem0.shape[1]
    F = B_w3.shape[1]
    SEG = int(A_seg_len)
    TB = 256
    NB = S // TB
    assert batch == 1 and DH == 128 and M == 8 and SEG % 16 == 0 and 2 * (M + SEG) <= DH
    assert S % TB == 0 and S % (2 * SEG) == 0 and D % (16 * NB) == 0 and H % 2 == 0
    out_dtype = A_x.dtype

    hbm = pl.BlockSpec(memory_space=pl.ANY)
    out = pl.pallas_call(
        functools.partial(_kernel, S=S, D=D, H=H, DH=DH, F=F, M=M, SEG=SEG, TB=TB),
        out_shape=jax.ShapeDtypeStruct((S, D), out_dtype),
        in_specs=[hbm, pl.BlockSpec(memory_space=pltpu.VMEM)] + [hbm] * 8,
        out_specs=hbm,
        scratch_shapes=[
            pltpu.VMEM((S, D), _BF16),
            pltpu.VMEM((S, D), out_dtype),
            pltpu.VMEM((S, D), _F32),
            pltpu.VMEM((S + 2 * _HALO, D), _F32),
            pltpu.VMEM((S, D), _F32),
            pltpu.VMEM((2, TB, D), _BF16),
            pltpu.VMEM((2, 7, TB // 2, D // 2), _BF16),
            pltpu.VMEM((D // 2, D), _U32),
            pltpu.VMEM((D // 2, D), _U32),
            pltpu.VMEM((D // 2, F), _U32),
            pltpu.VMEM((F // 2, D), _U32),
            pltpu.VMEM((3, D // 4, F // 2), _U32),
            pltpu.VMEM((3, F // 4, D // 2), _U32),
            pltpu.VMEM((NB, D // 2, 3 * H * DH // NB), _U32),
            pltpu.VMEM((H * DH // 2, D), _U32),
            pltpu.SemaphoreType.DMA((NB,)),
            pltpu.SemaphoreType.DMA((5,)),
            pltpu.SemaphoreType.DMA((NB,)),
            pltpu.SemaphoreType.DMA((1,)),
        ],
        compiler_params=pltpu.CompilerParams(vmem_limit_bytes=120 * 1024 * 1024),
    )(
        A_x.reshape(S, D),
        A_mem0.reshape(M, D),
        A_Wq.reshape(D // 2, 2, H, DH),
        A_Wk.reshape(D // 2, 2, H, DH),
        A_Wv.reshape(D // 2, 2, H, DH),
        A_Wo.reshape(H * DH, D),
        B_w1, B_w2, B_w3, B_w4,
    )
    return out.reshape(batch, S, D)
```

```python
import functools

import jax
import jax.numpy as jnp
from jax import lax
import jax.experimental.pallas as pl
import jax.experimental.pallas.tpu as pltpu

_EPS = 1e-5
_HALO = 8
_F32 = jnp.float32
_BF16 = jnp.bfloat16
_U32 = jnp.uint32


def _layernorm(v):
    m = jnp.mean(v, axis=-1, keepdims=True)
    c = v - m
    var = jnp.mean(c * c, axis=-1, keepdims=True)
    return c * lax.rsqrt(var + _EPS)


def _gelu(v):
    c = 0.7978845608028654
    h = 0.5 * v
    return h + h * jnp.tanh(v * (c + (c * 0.044715) * (v * v)))


def _silu(v):
    h = 0.5 * v
    return h + h * jnp.tanh(h)


def _dot(a, b):
    return jnp.dot(a, b, preferred_element_type=_F32)


def _dot_nt(a, b):
    return lax.dot_general(a, b, (((1,), (1,)), ((), ())), preferred_element_type=_F32)


def _strassen_lhs(a11, a12, a21, a22):
    sums = (a11 + a22, a21 + a22, a11, a22, a11 + a12, a21 - a11, a12 - a22)
    return [t.astype(_BF16) for t in sums]


def _strassen_dot(product):
    m5 = product(4)
    m3 = product(2)
    c12 = m3 + m5
    m4 = product(3)
    m2 = product(1)
    c21 = m2 + m4
    m1 = product(0)
    c11 = m4 - m5 + m1
    c22 = m3 - m2 + m1
    c11 = c11 + product(6)
    return c11, c12, c21, c22 + product(5)


def _kernel(
    x_hbm, mem0_hbm, wq_hbm, wk_hbm, wv_hbm, wo_hbm, w1_hbm, w2_hbm, w3_hbm, w4_hbm,
    out_hbm,
    x_v, o_v, mem0_v, xn_v, h_v, g_v, lhs_v, ls_v, w1_v, w2_v, w3_v, w4_v, e3_v, e4_v,
    wqkv_v, wo_v,
    sem_x, sem_w1, sem_w, sem_qkv, sem_out,
    *, S, D, H, DH, F, M, SEG, TB,
):
    NB = S // TB
    NP = H // 2
    PG = NP // NB
    L = M + SEG
    scale = DH ** (-0.5)

    def weights(ref):
        return pltpu.bitcast(ref, _BF16)

    def chunk(i, offset=0):
        return pl.ds(pl.multiple_of(i * TB + offset, 8), TB)

    def x_copy(i):
        rows = pl.ds(pl.multiple_of(i * TB, TB), TB)
        return pltpu.make_async_copy(x_hbm.at[rows], x_v.at[rows], sem_x.at[i])

    w_copies = [
        pltpu.make_async_copy(src, dst.bitcast(_BF16), sem_w.at[n])
        for n, (src, dst) in enumerate(
            ((w1_hbm, w1_v), (w2_hbm, w2_v), (w3_hbm, w3_v), (w4_hbm, w4_v), (wo_hbm, wo_v)))
    ]

    mem0_copy = pltpu.make_async_copy(mem0_hbm, mem0_v, sem_w.at[5])

    def start_group(i):
        for n, w in enumerate((wq_hbm, wk_hbm, wv_hbm)):
            w32 = w.bitcast(_U32)
            for p in range(PG):
                for parity in range(2):
                    c0 = (6 * p + 2 * n + parity) * DH
                    pltpu.make_async_copy(
                        w32.at[:, parity, i * PG + p, :],
                        wqkv_v.at[i, :, pl.ds(c0, DH)],
                        sem_qkv.at[i]).start()

    def repack(i):
        for c0 in range(0, 6 * PG * DH, 2 * DH):
            for r0 in range(0, D // 2, 8):
                rows = slice(r0, r0 + 8)
                ev = wqkv_v[i, rows, c0:c0 + DH]
                od = wqkv_v[i, rows, c0 + DH:c0 + 2 * DH]
                wqkv_v[i, rows, c0:c0 + DH] = (ev & _U32(0xFFFF)) | (od << 16)
                wqkv_v[i, rows, c0 + DH:c0 + 2 * DH] = (ev >> 16) | (od & _U32(0xFFFF0000))

    def out_copy(t):
        rows = pl.ds(pl.multiple_of(t * 2 * SEG, 2 * SEG), 2 * SEG)
        return pltpu.make_async_copy(o_v.at[rows], out_hbm.at[rows], sem_out.at[0])

    def w1_copy(q):
        cols = pl.ds(q * (D // 4), D // 4)
        return pltpu.make_async_copy(
            w1_hbm.at[:, cols], w1_v.bitcast(_BF16).at[:, cols], sem_w1.at[q])

    x_copy(0).start()
    for q in range(3):
        w1_copy(q).start()
    x_copy(1).start()
    w1_copy(3).start()
    for i in range(2, NB):
        x_copy(i).start()
    for cp in w_copies[1:4]:
        cp.start()

    zeros_halo = jnp.zeros((_HALO, D), _F32)
    h_v[pl.ds(0, _HALO), :] = zeros_halo
    h_v[pl.ds(_HALO + S, _HALO), :] = zeros_halo

    def norm_x(i, slot, r0=0, r1=TB):
        rows = pl.ds(pl.multiple_of(i * TB + r0, 16), r1 - r0)
        xn = _layernorm(x_v[rows, :].astype(_F32))
        xn_v[rows, :] = xn
        lhs_v[slot, r0:r1, :] = _layernorm(xn).astype(_BF16)

    def h_quarter(i, q):
        cols = slice(q * (D // 4), (q + 1) * (D // 4))
        h_v[chunk(i, _HALO), cols] = _gelu(_dot(lhs_v[i % 2], weights(w1_v[:, cols])))

    x_copy(0).wait()
    norm_x(0, 0)
    for q in range(4):
        w1_copy(q).wait()
        h_quarter(0, q)
        if q == 2:
            x_copy(1).wait()
            norm_x(1, 1)

    def phase1(i, carry):
        @pl.when(i + 1 < NB)
        def _():
            x_copy(i + 1).wait()

        cuts = (0, 80, 176, 256)
        for q in range(4):
            h_quarter(i, q)
            if q < 3:
                norm_x(jnp.minimum(i + 1, NB - 1), (i + 1) % 2, cuts[q], cuts[q + 1])
        return carry

    lax.fori_loop(1, NB, phase1, 0)

    def block_sum_jobs(w_v, i, parts):
        kh, nh = w_v.shape[0] // 2, w_v.shape[1] // 2
        nr = kh // parts
        for r in range(0, nr, 8):
            top = pl.ds(pl.multiple_of(i * nr + r, 8), 8)
            bot = pl.ds(pl.multiple_of(kh + i * nr + r, 8), 8)
            for c in range(0, nh, 128):
                yield top, bot, slice(c, c + 128), slice(nh + c, nh + c + 128)

    def block_sums(w_v, e_v, jobs, dep, zero):
        for top, bot, left, right in jobs:
            d = dep & zero
            b11, b12 = weights(w_v[top, left] | d), weights(w_v[top, right])
            b21, b22 = weights(w_v[bot, left]), weights(w_v[bot, right] | d)
            e_v[0, top, left] = pltpu.bitcast(b11 + b22, _U32)
            e_v[1, top, left] = pltpu.bitcast(b11 + b12, _U32)
            e_v[2, top, left] = pltpu.bitcast(b21 + b22, _U32)
            w_v[top, right] = pltpu.bitcast(b12 - b22, _U32)
            dep = pltpu.bitcast(b21 - b11, _U32)
            w_v[bot, left] = dep

    def strassen_rhs(w_v, e_v, k, r0, r1, c0, c1):
        kh, nh = w_v.shape[0] // 2, w_v.shape[1] // 2
        r0, r1 = r0 // 2, r1 // 2
        if k in (0, 5, 6):
            return weights(e_v[{0: 0, 5: 1, 6: 2}[k], r0:r1, c0:c1])
        dr, dc = {1: (0, 0), 2: (0, nh), 3: (kh, 0), 4: (kh, nh)}[k]
        return weights(w_v[dr + r0:dr + r1, dc + c0:dc + c1])

    def phase2a(w_v, e_v, first, i, carry):
        start_group(i)
        c = D // 4
        parts = []
        for q, shift in enumerate((-1, 1, -2, 2)):
            win = h_v[pl.ds(pl.multiple_of(i * TB, TB), TB + 2 * _HALO), q * c:(q + 1) * c]
            parts.append(win[_HALO + shift:_HALO + shift + TB].astype(_BF16))
        lhs = jnp.concatenate(parts, axis=1)
        zero = pltpu.bitcast(h_v[0:8, 0:128], _U32)
        jobs = list(block_sum_jobs(w_v, i - first, NB // 2))
        n = D // 8
        for q in range(8):
            cols = slice(q * n, (q + 1) * n)
            x1 = xn_v[chunk(i), cols] + _dot(lhs, weights(w2_v[:, cols]))
            g_v[chunk(i), cols] = x1
            if q < 8 - 1:
                part = jobs[q * len(jobs) // (8 - 1):(q + 1) * len(jobs) // (8 - 1)]
                block_sums(w_v, e_v, part, pltpu.bitcast(x1[:8, :128], _U32), zero)
        return carry

    w_copies[1].wait()
    w_copies[2].wait()
    lax.fori_loop(0, NB // 2, functools.partial(phase2a, w3_v, e3_v, 0), 0)
    w_copies[3].wait()
    lax.fori_loop(NB // 2, NB, functools.partial(phase2a, w4_v, e4_v, NB // 2), 0)
    w_copies[4].start()
    mem0_copy.start()

    HB, DHALF, FHALF = TB // 2, D // 2, F // 2

    def half(i, k, r0=0, r1=HB):
        return pl.ds(pl.multiple_of(i * TB + k * HB + r0, 16), r1 - r0)

    def norm_x1(i, slot, r0=0, r1=HB):
        top = _layernorm(g_v[half(i, 0, r0, r1), :])
        bot = _layernorm(g_v[half(i, 1, r0, r1), :])
        ops = _strassen_lhs(top[:, :DHALF], top[:, DHALF:], bot[:, :DHALF], bot[:, DHALF:])
        for k in range(7):
            ls_v[slot, k, r0:r1, :] = ops[k]

    norm_x1(0, 0)

    def phase2b(i, carry):
        pltpu.make_async_copy(wqkv_v.at[i], wqkv_v.at[i], sem_qkv.at[i]).wait()
        us = []
        for n, c0 in enumerate(range(0, FHALF, 256)):
            pre = _strassen_dot(lambda k: _dot(
                ls_v[i % 2, k], strassen_rhs(w3_v, e3_v, k, 0, DHALF, c0, c0 + 256)))
            us.append(_strassen_lhs(*[_gelu(t) for t in pre]))
            m = n * 256 // 256
            if (n * 256) % 256 == 0 and m < 4:
                norm_x1(jnp.minimum(i + 1, NB - 1), (i + 1) % 2, m * HB // 4, (m + 1) * HB // 4)
        u = [jnp.concatenate([t[k] for t in us], axis=1) for k in range(7)]
        cut = FHALF - 512
        first = (0, 256, 384, 512)[1]
        head = {k: _dot(u[k][:, :cut], strassen_rhs(w4_v, e4_v, k, 0, cut, 0, first))
                for k in (4, 2, 3)}
        for c0, c1 in zip((0, 256, 384, 512)[:-1], (0, 256, 384, 512)[1:]):
            def product(k):
                if k in head:
                    return head.pop(k) + _dot(
                        u[k][:, cut:], strassen_rhs(w4_v, e4_v, k, cut, FHALF, c0, c1))
                return _dot(u[k], strassen_rhs(w4_v, e4_v, k, 0, FHALF, c0, c1))
            for n, y in enumerate(_strassen_dot(product)):
                rows = half(i, n // 2)
                cols = slice((n % 2) * DHALF + c0, (n % 2) * DHALF + c1)
                g_v[rows, cols] = _silu(g_v[rows, cols] + y)
        repack(i)
        return carry

    lax.fori_loop(0, NB, phase2b, 0)
    w_copies[4].wait()
    mem0_copy.wait()

    row = lax.broadcasted_iota(jnp.int32, (2 * L, DH), 0)
    col = lax.broadcasted_iota(jnp.int32, (2 * L, DH), 1)
    rl = jnp.where(row >= L, row - L, row)
    cl = jnp.where(col >= L, col - L, col)
    same_head = ((row >= L) == (col >= L)) & (col < 2 * L)
    visible = same_head & ((rl < M) | (rl >= cl))
    fill = jnp.where(same_head, -1e9, -jnp.inf).astype(_F32)
    pad = jnp.zeros((DH - 2 * L, DH), _BF16)

    def project(lhs, j):
        c0 = 6 * (j % PG) * DH
        return _dot(lhs, weights(wqkv_v[j // PG, :, c0:c0 + 6 * DH]))

    def pair(r, n):
        return jnp.concatenate(
            [r[:, 2 * n * DH:(2 * n + 1) * DH], r[:, (2 * n + 1) * DH:(2 * n + 2) * DH]],
            axis=0).astype(_BF16)

    def scores(r):
        s = _dot_nt(pair(r, 0), jnp.concatenate([pair(r, 1), pad], axis=0))
        return s, jnp.concatenate([pair(r, 2), pad], axis=0)

    def attend(s, v):
        z = jnp.where(visible, s * scale, fill)
        e = jnp.exp(z - jnp.max(z, axis=-1, keepdims=True))
        p = e / jnp.sum(e, axis=-1, keepdims=True)
        o = _dot(p.astype(_BF16), v)
        return jnp.concatenate([o[:L], o[L:]], axis=1)

    def out_proj(o, j0, j1, n0, n1):
        return _dot(o, weights(wo_v[j0 * DH:j1 * DH, n0:n1]))

    def step(lhs, seq_rows, out_rows):
        LAG = 3
        early = NP - LAG
        nw = D // (LAG + 1)
        rs, sv, os_, ys = {}, {}, [], []
        for j in range(NP + LAG + 1):
            if j < NP:
                rs[j] = seq_rows(j, project(lhs, j))
            else:
                if j == NP:
                    o_early = jnp.concatenate(os_[:early], axis=1)
                ys.append(out_proj(o_early, 0, early, (j - NP) * nw, (j - NP + 1) * nw))
            if LAG <= j < NP + LAG:
                os_.append(out_rows(j - LAG, attend(*sv.pop(j - LAG))).astype(_BF16))
            if 1 <= j <= NP:
                sv[j - 1] = scores(rs.pop(j - 1))
        o_late = jnp.concatenate(os_[early:], axis=1)
        return jnp.concatenate(ys, axis=1) + out_proj(o_late, early, NP, 0, D)

    A = SEG + M
    B = SEG - M

    def phase3(t, mem):
        base = pl.multiple_of(t * 2 * SEG, 2 * SEG)
        held_r, held_o = {}, {}

        def seq_even(j, r):
            held_r[j] = r[L:]
            return r[:L]

        def out_even(j, o):
            held_o[j] = o[M + B:]
            return o[:M + B]

        def seq_odd(j, r):
            return jnp.concatenate([r[:M], held_r[j], r[M:]], axis=0)

        def out_odd(j, o):
            return jnp.concatenate([o[:M], held_o[j], o[M:]], axis=0)

        lhs0 = jnp.concatenate([mem, xn_v[pl.ds(base, A), :]], axis=0).astype(_BF16)
        y0 = step(lhs0, seq_even, out_even)
        rest = pl.ds(pl.multiple_of(base + A, 8), 2 * SEG - A)
        lhs1 = jnp.concatenate([y0[:M], xn_v[rest, :]], axis=0).astype(_BF16)
        y1 = step(lhs1, seq_odd, out_odd)

        rows = pl.ds(base, 2 * SEG)
        s = jnp.concatenate([y0[M:], y1[M:]], axis=0)
        o_v[rows, :] = (x_v[rows, :].astype(_F32) + s * g_v[rows, :]).astype(o_v.dtype)
        out_copy(t).start()
        return y1[:M]

    lax.fori_loop(0, S // (2 * SEG), phase3, mem0_v[...].astype(_F32))
    pltpu.make_async_copy(o_v, out_hbm, sem_out.at[0]).wait()


@functools.partial(jax.jit, static_argnames=("A_seg_len",))
def pallas_recurrent_scan__memory_aug_recurrent_mem_tr__mixer_s_mlp__prompt_kernel(
    A_x: jax.Array,
    A_mem0: jax.Array,
    A_Wq: jax.Array,
    A_Wk: jax.Array,
    A_Wv: jax.Array,
    A_Wo: jax.Array,
    A_seg_len: int,
    B_x: jax.Array,
    B_w1: jax.Array,
    B_w2: jax.Array,
    B_w3: jax.Array,
    B_w4: jax.Array,
):
    del B_x
    batch, S, D = A_x.shape
    _, H, DH = A_Wq.shape
    M = A_mem0.shape[1]
    F = B_w3.shape[1]
    SEG = int(A_seg_len)
    TB = 256
    NB = S // TB
    assert batch == 1 and DH == 128 and M == 8 and SEG % 16 == 0 and 2 * (M + SEG) <= DH
    assert S % TB == 0 and S % (2 * SEG) == 0 and D % (16 * NB) == 0 and H % 2 == 0
    out_dtype = A_x.dtype

    hbm = pl.BlockSpec(memory_space=pl.ANY)
    out = pl.pallas_call(
        functools.partial(_kernel, S=S, D=D, H=H, DH=DH, F=F, M=M, SEG=SEG, TB=TB),
        out_shape=jax.ShapeDtypeStruct((S, D), out_dtype),
        in_specs=[hbm] * 10,
        out_specs=hbm,
        scratch_shapes=[
            pltpu.VMEM((S, D), _BF16),
            pltpu.VMEM((S, D), out_dtype),
            pltpu.VMEM((M, D), A_mem0.dtype),
            pltpu.VMEM((S, D), _F32),
            pltpu.VMEM((S + 2 * _HALO, D), _F32),
            pltpu.VMEM((S, D), _F32),
            pltpu.VMEM((2, TB, D), _BF16),
            pltpu.VMEM((2, 7, TB // 2, D // 2), _BF16),
            pltpu.VMEM((D // 2, D), _U32),
            pltpu.VMEM((D // 2, D), _U32),
            pltpu.VMEM((D // 2, F), _U32),
            pltpu.VMEM((F // 2, D), _U32),
            pltpu.VMEM((3, D // 4, F // 2), _U32),
            pltpu.VMEM((3, F // 4, D // 2), _U32),
            pltpu.VMEM((NB, D // 2, 3 * H * DH // NB), _U32),
            pltpu.VMEM((H * DH // 2, D), _U32),
            pltpu.SemaphoreType.DMA((NB,)),
            pltpu.SemaphoreType.DMA((4,)),
            pltpu.SemaphoreType.DMA((6,)),
            pltpu.SemaphoreType.DMA((NB,)),
            pltpu.SemaphoreType.DMA((1,)),
        ],
        compiler_params=pltpu.CompilerParams(vmem_limit_bytes=120 * 1024 * 1024),
    )(
        A_x.reshape(S, D),
        A_mem0.reshape(M, D),
        A_Wq.reshape(D // 2, 2, H, DH),
        A_Wk.reshape(D // 2, 2, H, DH),
        A_Wv.reshape(D // 2, 2, H, DH),
        A_Wo.reshape(H * DH, D),
        B_w1, B_w2, B_w3, B_w4,
    )
    return out.reshape(batch, S, D)
```

```python
import functools

import jax
import jax.numpy as jnp
from jax import lax
import jax.experimental.pallas as pl
import jax.experimental.pallas.tpu as pltpu

_EPS = 1e-5
_HALO = 8
_TB = 256
_F32 = jnp.float32
_BF16 = jnp.bfloat16
_U32 = jnp.uint32


def _layernorm(v):
    m = jnp.mean(v, axis=-1, keepdims=True)
    c = v - m
    var = jnp.mean(c * c, axis=-1, keepdims=True)
    return c * lax.rsqrt(var + _EPS)


def _gelu(v):
    c = 0.7978845608028654
    h = 0.5 * v
    return h + h * jnp.tanh(v * (c + (c * 0.044715) * (v * v)))


def _silu(v):
    h = 0.5 * v
    return h + h * jnp.tanh(h)


def _dot(a, b):
    return jnp.dot(a, b, preferred_element_type=_F32)


def _dot_nt(a, b):
    return lax.dot_general(a, b, (((1,), (1,)), ((), ())), preferred_element_type=_F32)


def _rows(words):
    return pltpu.bitcast(words, _BF16)


def _words(rows):
    return pltpu.bitcast(rows, _U32)


def _strassen_lhs(a11, a12, a21, a22):
    sums = (a11 + a22, a21 + a22, a11, a22, a11 + a12, a21 - a11, a12 - a22)
    return [t.astype(_BF16) for t in sums]


def _strassen_dot(product):
    m5 = product(4)
    m3 = product(2)
    c12 = m3 + m5
    m4 = product(3)
    m2 = product(1)
    c21 = m2 + m4
    m1 = product(0)
    c11 = m4 - m5 + m1
    c22 = m3 - m2 + m1
    c11 = c11 + product(6)
    return c11, c12, c21, c22 + product(5)


def _kernel(
    x_hbm, mem0_hbm, wq_hbm, wk_hbm, wv_hbm, wo_hbm, w1_hbm, w2_hbm, w3_hbm, w4_hbm,
    out_hbm,
    x_v, o_v, mem0_v, xn_v, h_v, g_v, lhs_v, ls_v,
    w1_v, w2_v, w3_v, w4_v, e3_v, e4_v, wqkv_v, wo_v,
    sem_x, sem_w1, sem_w, sem_qkv, sem_out,
    *, S, D, H, DH, F, M, SEG,
):
    TB = _TB
    NB = S // TB
    NP = H // 2
    PG = NP // NB
    L = M + SEG
    DQ = D // 4

    def chunk(i, offset=0):
        return pl.ds(pl.multiple_of(i * TB + offset, 8), TB)

    def x_copy(i):
        return pltpu.make_async_copy(x_hbm.at[chunk(i)], x_v.at[chunk(i)], sem_x.at[i])

    def w1_copy(q):
        cols = pl.ds(q * DQ, DQ)
        return pltpu.make_async_copy(
            w1_hbm.bitcast(_U32).at[:, cols], w1_v.at[:, cols], sem_w1.at[q])

    w2_copy, w3_copy, w4_copy, wo_copy = (
        pltpu.make_async_copy(src.bitcast(_U32), dst, sem_w.at[n])
        for n, (src, dst) in enumerate(
            ((w2_hbm, w2_v), (w3_hbm, w3_v), (w4_hbm, w4_v), (wo_hbm, wo_v))))
    mem0_copy = pltpu.make_async_copy(mem0_hbm, mem0_v, sem_w.at[4])

    def start_group(i):
        for n, w in enumerate((wq_hbm, wk_hbm, wv_hbm)):
            for p in range(PG):
                for parity in range(2):
                    pltpu.make_async_copy(
                        w.bitcast(_U32).at[:, parity, i * PG + p, :],
                        wqkv_v.at[i, :, pl.ds((6 * p + 2 * n + parity) * DH, DH)],
                        sem_qkv.at[i]).start()

    def wait_group(i):
        pltpu.make_async_copy(wqkv_v.at[i], wqkv_v.at[i], sem_qkv.at[i]).wait()

    def repack(i):
        for c0 in range(0, 6 * PG * DH, 2 * DH):
            lo, hi = slice(c0, c0 + DH), slice(c0 + DH, c0 + 2 * DH)
            for r0 in range(0, D // 2, 8):
                rows = slice(r0, r0 + 8)
                ev, od = wqkv_v[i, rows, lo], wqkv_v[i, rows, hi]
                wqkv_v[i, rows, lo] = (ev & _U32(0xFFFF)) | (od << 16)
                wqkv_v[i, rows, hi] = (ev >> 16) | (od & _U32(0xFFFF0000))

    def out_copy(t):
        rows = pl.ds(pl.multiple_of(t * 2 * SEG, 2 * SEG), 2 * SEG)
        return pltpu.make_async_copy(o_v.at[rows], out_hbm.at[rows], sem_out.at[0])

    x_copy(0).start()
    for q in range(3):
        w1_copy(q).start()
    x_copy(1).start()
    w1_copy(3).start()
    for i in range(2, NB):
        x_copy(i).start()
    w2_copy.start()
    w3_copy.start()
    w4_copy.start()

    h_v[pl.ds(0, _HALO), :] = jnp.zeros((_HALO, D), _F32)
    h_v[pl.ds(_HALO + S, _HALO), :] = jnp.zeros((_HALO, D), _F32)

    def norm_x(i, slot, r0=0, r1=TB):
        rows = pl.ds(pl.multiple_of(i * TB + r0, 16), r1 - r0)
        xn = _layernorm(x_v[rows, :].astype(_F32))
        xn_v[rows, :] = xn
        lhs_v[slot, r0:r1, :] = _layernorm(xn).astype(_BF16)

    def h_quarter(i, q):
        cols = slice(q * DQ, (q + 1) * DQ)
        h_v[chunk(i, _HALO), cols] = _gelu(_dot(lhs_v[i % 2], _rows(w1_v[:, cols])))

    x_copy(0).wait()
    norm_x(0, 0)
    for q in range(4):
        w1_copy(q).wait()
        h_quarter(0, q)
        if q == 2:
            x_copy(1).wait()
            norm_x(1, 1)

    def phase1(i, carry):
        @pl.when(i + 1 < NB)
        def _():
            x_copy(i + 1).wait()

        cuts = (0, 80, 176, TB)
        for q in range(4):
            h_quarter(i, q)
            if q < 3:
                norm_x(jnp.minimum(i + 1, NB - 1), (i + 1) % 2, cuts[q], cuts[q + 1])
        return carry

    lax.fori_loop(1, NB, phase1, 0)

    def block_sum_jobs(w_v, i, parts):
        kh, nh = w_v.shape[0] // 2, w_v.shape[1] // 2
        nr = kh // parts
        for r in range(0, nr, 8):
            top = pl.ds(pl.multiple_of(i * nr + r, 8), 8)
            bot = pl.ds(pl.multiple_of(kh + i * nr + r, 8), 8)
            for c in range(0, nh, 128):
                yield top, bot, slice(c, c + 128), slice(nh + c, nh + c + 128)

    def block_sums(w_v, e_v, jobs, after, zero):
        for top, bot, left, right in jobs:
            nil = after & zero
            b11, b12 = _rows(w_v[top, left] | nil), _rows(w_v[top, right])
            b21, b22 = _rows(w_v[bot, left]), _rows(w_v[bot, right] | nil)
            e_v[0, top, left] = _words(b11 + b22)
            e_v[1, top, left] = _words(b11 + b12)
            e_v[2, top, left] = _words(b21 + b22)
            w_v[top, right] = _words(b12 - b22)
            after = _words(b21 - b11)
            w_v[bot, left] = after

    def strassen_rhs(w_v, e_v, k, r0, r1, c0, c1):
        kh, nh = w_v.shape[0] // 2, w_v.shape[1] // 2
        r0, r1 = r0 // 2, r1 // 2
        if k in (0, 5, 6):
            return _rows(e_v[(0, 5, 6).index(k), r0:r1, c0:c1])
        dr, dc = ((0, 0), (0, nh), (kh, 0), (kh, nh))[k - 1]
        return _rows(w_v[dr + r0:dr + r1, dc + c0:dc + c1])

    def phase2a(w_v, e_v, first, i, carry):
        start_group(i)
        parts = []
        for q, shift in enumerate((-1, 1, -2, 2)):
            rows = pl.ds(pl.multiple_of(i * TB, TB), TB + 2 * _HALO)
            win = h_v[rows, q * DQ:(q + 1) * DQ]
            parts.append(win[_HALO + shift:_HALO + shift + TB].astype(_BF16))
        lhs = jnp.concatenate(parts, axis=1)
        zero = pltpu.bitcast(h_v[0:_HALO, 0:128], _U32)
        jobs = list(block_sum_jobs(w_v, i - first, NB // 2))
        nt = D // 128
        for q in range(nt):
            cols = slice(q * 128, (q + 1) * 128)
            x1 = xn_v[chunk(i), cols] + _dot(lhs, _rows(w2_v[:, cols]))
            g_v[chunk(i), cols] = x1
            if q < nt - 1:
                part = jobs[q * len(jobs) // (nt - 1):(q + 1) * len(jobs) // (nt - 1)]
                block_sums(w_v, e_v, part, pltpu.bitcast(x1[:8], _U32), zero)
        return carry

    w2_copy.wait()
    w3_copy.wait()
    lax.fori_loop(0, NB // 2, functools.partial(phase2a, w3_v, e3_v, 0), 0)
    w4_copy.wait()
    lax.fori_loop(NB // 2, NB, functools.partial(phase2a, w4_v, e4_v, NB // 2), 0)
    wo_copy.start()
    mem0_copy.start()

    TH, DHALF, FHALF = TB // 2, D // 2, F // 2

    def half(i, k, r0=0, r1=TH):
        return pl.ds(pl.multiple_of(i * TB + k * TH + r0, 16), r1 - r0)

    def norm_x1(i, slot, r0=0, r1=TH):
        top = _layernorm(g_v[half(i, 0, r0, r1), :])
        bot = _layernorm(g_v[half(i, 1, r0, r1), :])
        ops = _strassen_lhs(top[:, :DHALF], top[:, DHALF:], bot[:, :DHALF], bot[:, DHALF:])
        for k in range(7):
            ls_v[slot, k, r0:r1, :] = ops[k]

    norm_x1(0, 0)

    def phase2b(i, carry):
        wait_group(i)
        us = []
        for n, c0 in enumerate(range(0, FHALF, 256)):
            pre = _strassen_dot(lambda k: _dot(
                ls_v[i % 2, k], strassen_rhs(w3_v, e3_v, k, 0, DHALF, c0, c0 + 256)))
            us.append(_strassen_lhs(*[_gelu(t) for t in pre]))
            if n < 4:
                norm_x1(jnp.minimum(i + 1, NB - 1), (i + 1) % 2,
                        n * TH // 4, (n + 1) * TH // 4)
        u = [jnp.concatenate([t[k] for t in us], axis=1) for k in range(7)]

        cut = FHALF - 512
        cuts = (0, DHALF // 2, 3 * DHALF // 4, DHALF)
        head = {k: _dot(u[k][:, :cut], strassen_rhs(w4_v, e4_v, k, 0, cut, 0, cuts[1]))
                for k in (4, 2, 3)}
        for c0, c1 in zip(cuts[:-1], cuts[1:]):
            def product(k):
                if k in head:
                    return head.pop(k) + _dot(
                        u[k][:, cut:], strassen_rhs(w4_v, e4_v, k, cut, FHALF, c0, c1))
                return _dot(u[k], strassen_rhs(w4_v, e4_v, k, 0, FHALF, c0, c1))

            for n, y in enumerate(_strassen_dot(product)):
                rows = half(i, n // 2)
                cols = slice((n % 2) * DHALF + c0, (n % 2) * DHALF + c1)
                g_v[rows, cols] = _silu(g_v[rows, cols] + y)
        repack(i)
        return carry

    lax.fori_loop(0, NB, phase2b, 0)
    wo_copy.wait()
    mem0_copy.wait()

    row = lax.broadcasted_iota(jnp.int32, (2 * L, DH), 0)
    col = lax.broadcasted_iota(jnp.int32, (2 * L, DH), 1)
    rl = jnp.where(row >= L, row - L, row)
    cl = jnp.where(col >= L, col - L, col)
    same_head = ((row >= L) == (col >= L)) & (col < 2 * L)
    visible = same_head & ((rl < M) | (rl >= cl))
    fill = jnp.where(same_head, -1e9, -jnp.inf).astype(_F32)
    pad = jnp.zeros((DH - 2 * L, DH), _BF16)

    def project(lhs, j):
        c0 = 6 * (j % PG) * DH
        return _dot(lhs, _rows(wqkv_v[j // PG, :, c0:c0 + 6 * DH]))

    def pair(r, n):
        return jnp.concatenate(
            [r[:, 2 * n * DH:(2 * n + 1) * DH], r[:, (2 * n + 1) * DH:(2 * n + 2) * DH]],
            axis=0).astype(_BF16)

    def scores(r):
        s = _dot_nt(pair(r, 0), jnp.concatenate([pair(r, 1), pad], axis=0))
        return s, jnp.concatenate([pair(r, 2), pad], axis=0)

    def attend(s, v):
        z = jnp.where(visible, s * DH ** (-0.5), fill)
        e = jnp.exp(z - jnp.max(z, axis=-1, keepdims=True))
        p = e / jnp.sum(e, axis=-1, keepdims=True)
        o = _dot(p.astype(_BF16), v)
        return jnp.concatenate([o[:L], o[L:]], axis=1)

    def out_proj(o, j0, j1, c0, c1):
        return _dot(o, _rows(wo_v[j0 * DH:j1 * DH, c0:c1]))

    def step(lhs, seq_rows, out_rows):
        lag = 3
        early = NP - lag
        cuts = (0, D // 8, 3 * D // 8, 5 * D // 8, D)
        rs, sv, os_, ys = {}, {}, [], []
        for j in range(NP + lag + 1):
            if j < NP:
                rs[j] = seq_rows(j, project(lhs, j))
            else:
                ys.append(out_proj(jnp.concatenate(os_[:early], axis=1), 0, early,
                                   cuts[j - NP], cuts[j - NP + 1]))
            if lag <= j < NP + lag:
                os_.append(out_rows(j - lag, attend(*sv.pop(j - lag))).astype(_BF16))
            if 1 <= j <= NP:
                sv[j - 1] = scores(rs.pop(j - 1))
        late = out_proj(jnp.concatenate(os_[early:], axis=1), early, NP, 0, D)
        return jnp.concatenate(ys, axis=1) + late

    def phase3(t, mem):
        base = pl.multiple_of(t * 2 * SEG, 2 * SEG)
        held_r, held_o = {}, {}

        def seq_even(j, r):
            held_r[j] = r[L:]
            return r[:L]

        def out_even(j, o):
            held_o[j] = o[SEG:]
            return o[:SEG]

        def seq_odd(j, r):
            return jnp.concatenate([r[:M], held_r[j], r[M:]], axis=0)

        def out_odd(j, o):
            return jnp.concatenate([o[:M], held_o[j], o[M:]], axis=0)

        lhs0 = jnp.concatenate([mem, xn_v[pl.ds(base, L), :]], axis=0)
        y0 = step(lhs0.astype(_BF16), seq_even, out_even)
        rest = pl.ds(pl.multiple_of(base + L, 8), SEG - M)
        lhs1 = jnp.concatenate([y0[:M], xn_v[rest, :]], axis=0)
        y1 = step(lhs1.astype(_BF16), seq_odd, out_odd)

        rows = pl.ds(base, 2 * SEG)
        s = jnp.concatenate([y0[M:], y1[M:]], axis=0)
        o_v[rows, :] = (x_v[rows, :].astype(_F32) + s * g_v[rows, :]).astype(o_v.dtype)
        out_copy(t).start()
        return y1[:M]

    lax.fori_loop(0, S // (2 * SEG), phase3, mem0_v[...].astype(_F32))
    pltpu.make_async_copy(o_v, out_hbm, sem_out.at[0]).wait()


@functools.partial(jax.jit, static_argnames=("A_seg_len",))
def pallas_recurrent_scan__memory_aug_recurrent_mem_tr__mixer_s_mlp__prompt_kernel(
    A_x: jax.Array,
    A_mem0: jax.Array,
    A_Wq: jax.Array,
    A_Wk: jax.Array,
    A_Wv: jax.Array,
    A_Wo: jax.Array,
    A_seg_len: int,
    B_x: jax.Array,
    B_w1: jax.Array,
    B_w2: jax.Array,
    B_w3: jax.Array,
    B_w4: jax.Array,
):
    del B_x
    batch, S, D = A_x.shape
    _, H, DH = A_Wq.shape
    M = A_mem0.shape[1]
    F = B_w3.shape[1]
    SEG = int(A_seg_len)
    NB = S // _TB
    assert batch == 1 and DH == 128 and M == 8 and D % 1024 == 0 and F % 512 == 0
    assert SEG % 16 == 0 and 2 * (M + SEG) <= DH and S % (2 * SEG) == 0
    assert S % _TB == 0 and NB % 2 == 0 and H % (2 * NB) == 0 and F >= 2048
    assert all(a.dtype == _BF16 for a in (A_x, A_Wq, A_Wk, A_Wv, A_Wo, B_w1, B_w2, B_w3, B_w4))

    hbm = pl.BlockSpec(memory_space=pl.ANY)
    out = pl.pallas_call(
        functools.partial(_kernel, S=S, D=D, H=H, DH=DH, F=F, M=M, SEG=SEG),
        out_shape=jax.ShapeDtypeStruct((S, D), A_x.dtype),
        in_specs=[hbm] * 10,
        out_specs=hbm,
        scratch_shapes=[
            pltpu.VMEM((S, D), A_x.dtype),
            pltpu.VMEM((S, D), A_x.dtype),
            pltpu.VMEM((M, D), A_mem0.dtype),
            pltpu.VMEM((S, D), _F32),
            pltpu.VMEM((S + 2 * _HALO, D), _F32),
            pltpu.VMEM((S, D), _F32),
            pltpu.VMEM((2, _TB, D), _BF16),
            pltpu.VMEM((2, 7, _TB // 2, D // 2), _BF16),
            pltpu.VMEM((D // 2, D), _U32),
            pltpu.VMEM((D // 2, D), _U32),
            pltpu.VMEM((D // 2, F), _U32),
            pltpu.VMEM((F // 2, D), _U32),
            pltpu.VMEM((3, D // 4, F // 2), _U32),
            pltpu.VMEM((3, F // 4, D // 2), _U32),
            pltpu.VMEM((NB, D // 2, 3 * H * DH // NB), _U32),
            pltpu.VMEM((H * DH // 2, D), _U32),
            pltpu.SemaphoreType.DMA((NB,)),
            pltpu.SemaphoreType.DMA((4,)),
            pltpu.SemaphoreType.DMA((5,)),
            pltpu.SemaphoreType.DMA((NB,)),
            pltpu.SemaphoreType.DMA((1,)),
        ],
        compiler_params=pltpu.CompilerParams(vmem_limit_bytes=120 * 1024 * 1024),
    )(
        A_x.reshape(S, D),
        A_mem0.reshape(M, D),
        A_Wq.reshape(D // 2, 2, H, DH),
        A_Wk.reshape(D // 2, 2, H, DH),
        A_Wv.reshape(D // 2, 2, H, DH),
        A_Wo.reshape(H * DH, D),
        B_w1, B_w2, B_w3, B_w4,
    )
    return out.reshape(batch, S, D)
```
